```python
import jax
import jax.numpy as jnp

def _softmax(x, axis=-1):
    return jax.nn.softmax(x, axis=axis)
def _gelu(x):
    return jax.nn.gelu(x, approximate=True)
def _silu(x):
    return jax.nn.silu(x)
def _sigmoid(x):
    return jax.nn.sigmoid(x)
def _layernorm(x, axis=-1, eps=1e-5):
    m = jnp.mean(x, axis=axis, keepdims=True)
    v = jnp.var(x, axis=axis, keepdims=True)
    return (x - m) / jnp.sqrt(v + eps)
def _scatter_add(tgt, idx, src, axis=0):
    return tgt.at[idx].add(src)
def _segment_sum(src, seg, n):
    return jax.ops.segment_sum(src, seg, n)
class _Rng:
    def __init__(self, key):
        self._k = key
    def _next(self):
        self._k, sub = jax.random.split(self._k)
        return sub
    def normal(self, shape):
        return jax.random.normal(self._next(), shape, dtype=jnp.bfloat16)
    def randint(self, lo, hi, shape):
        return jax.random.randint(self._next(), shape, lo, hi, dtype=jnp.int32)
    def uniform(self, shape, lo=0.0, hi=1.0):
        return jax.random.uniform(self._next(), shape, jnp.bfloat16, lo, hi)
    def permutation(self, n):
        return jax.random.permutation(self._next(), n)


kernel_name = 'standalone__modern_conv_block_convnext__vision'

def setup_inputs():
    _rng = _Rng(jax.random.key(int.from_bytes(__import__("os").urandom(4), "little")))
    _w = (lambda a: (lambda t: t.astype(jnp.bfloat16) if jnp.issubdtype(t.dtype, jnp.floating) else t)(jnp.asarray(a)))
    H = W = 512
    C = 96
    K = 3
    return {
        "x": _w((lambda *s: _rng.normal(s) * 0.05)(1, H, W, C)),
        "dw": _w((lambda *s: _rng.normal(s) * 0.05)(K, K, C)),
        "w1": _w((lambda *s: _rng.normal(s) * 0.05)(C, 4 * C)),
        "b1": _w((lambda *s: _rng.normal(s) * 0.05)(4 * C)),
        "w2": _w((lambda *s: _rng.normal(s) * 0.05)(4 * C, C)),
        "b2": _w((lambda *s: _rng.normal(s) * 0.05)(C)),
        "gamma": _w((lambda *s: _rng.normal(s) * 0.05)(C)),
    }

def reference(x, dw, w1, b1, w2, b2, gamma):
    B, H, W, C = x.shape
    K = dw.shape[0]
    pad = K // 2
    xp = jnp.pad(x, ((0,0),(pad,pad),(pad,pad),(0,0)))
    out = jnp.zeros_like(x)
    for i in range(K):
        for j in range(K):
            out = out + xp[:, i:i+H, j:j+W, :] * dw[i, j][None, None, None, :]
    h = _layernorm(out, axis=-1)
    h = jnp.einsum('bhwc,ce->bhwe', h, w1) + b1
    h = _gelu(h)
    h = jnp.einsum('bhwe,ec->bhwc', h, w2) + b2
    return x + gamma[None, None, None, :] * h
```

```python
import functools
import jax
import jax.numpy as jnp
from jax import lax
import jax.experimental.pallas as pl
import jax.experimental.pallas.tpu as pltpu
import numpy as np

_K0 = float(np.sqrt(2.0 / np.pi))
_K1 = _K0 * 0.044715
_A = _K1 ** (1.0 / 3.0)
_C0 = _K0 / _A
_EPS = 1e-5
F32 = jnp.float32
BF16 = jnp.bfloat16
U32 = jnp.uint32


def _make(H, C, W, E, U, o):
    NBLK = H // U
    NT = W // 128
    NCG = C // 8
    NK = E // 128
    NUP = 6
    WINO = 0
    NWT = 12 if WINO else 9
    XL = o.get('xl', 1) + WINO
    LA = U + 2 + XL
    RING = 4 * U
    NXB = 4
    NOB = 4
    HW = W // 2
    NRP = o.get('nrp', 4)
    MODE = o.get('mode', 3)
    assert NBLK % 2 == 0

    def kernel(x_hbm, dw_ref, w1_ref, b1_ref, w2t_ref, b2_ref, g_ref, o_hbm,
               xbuf, obuf, xsem, osem, w1s, w2s, xf, ya, yb, accx, gs, zs):

        def xchunk(k):
            s_ = k % NXB
            return pltpu.make_async_copy(x_hbm.at[pl.ds(k * U + LA, U)], xbuf.at[s_], xsem.at[s_])

        KP = (H - LA) // U
        NP = H - LA - KP * U

        def xpart():
            return pltpu.make_async_copy(x_hbm.at[pl.ds(H - NP, NP)], xbuf.at[KP % NXB, pl.ds(0, NP)], xsem.at[KP % NXB])

        def ochunk(k):
            s_ = k % NOB
            return pltpu.make_async_copy(obuf.at[s_], o_hbm.at[pl.ds(k * U - 1, U)], osem.at[s_])

        ofirst = pltpu.make_async_copy(obuf.at[0, pl.ds(1, U - 1)], o_hbm.at[pl.ds(0, U - 1)], osem.at[0])
        olast = pltpu.make_async_copy(obuf.at[NBLK % NOB, pl.ds(0, 1)], o_hbm.at[pl.ds(H - 1, 1)], osem.at[NBLK % NOB])

        def tiles(v):
            return [v[:, t * 128:(t + 1) * 128] for t in range(NT)]

        def wtap(ref, k, cs):
            return ref[RING + k // 4, cs, (k % 4) * 128:(k % 4) * 128 + 128]

        def conv_piece(cg, x0, x1, x2, wref, want_z=False, wino=False):
            lane = lax.broadcasted_iota(jnp.int32, (8, 128), 1)
            cs = slice(cg * 8, cg * 8 + 8)
            wv = [wtap(wref, k, cs) for k in range(9)]
            x0, x1, x2 = tiles(x0), tiles(x1), tiles(x2)
            z = [[x0[t] * wv[b] + x1[t] * wv[3 + b] + x2[t] * wv[6 + b] for t in range(NT)] for b in range(3)]
            if o.get('casc', 0):
                L1 = [pltpu.roll(v, 127, 1) for v in z[1]]
                L2 = [pltpu.roll(v, 127, 1) for v in z[2]]
                bb = [z[0][t] + jnp.where(lane == 127, L1[t + 1] if t < NT - 1 else 0.0, L1[t]) for t in range(NT)]
                Rb = [pltpu.roll(v, 1, 1) for v in bb]
                out = [jnp.where(lane == 0, Rb[t - 1] if t > 0 else z[1][0], Rb[t])
                       + jnp.where(lane == 127, L2[t + 1] if t < NT - 1 else 0.0, L2[t]) for t in range(NT)]
            else:
                Rr = [pltpu.roll(v, 1, 1) for v in z[0]]
                Ll = [pltpu.roll(v, 127, 1) for v in z[2]]
                out = []
                for t in range(NT):
                    lt = jnp.where(lane == 0, Rr[t - 1] if t > 0 else 0.0, Rr[t])
                    rt = jnp.where(lane == 127, Ll[t + 1] if t < NT - 1 else 0.0, Ll[t])
                    out.append(z[1][t] + lt + rt)
            return (out, z) if want_z else out

        def wino_front(cg, d, wref):
            cs = slice(cg * 8, cg * 8 + 8)
            wv = [wtap(wref, k, cs) for k in range(12)]
            n = d[0].shape[1] // 128
            d = [[v[:, t * 128:(t + 1) * 128] for t in range(n)] for v in d]
            T = [(d[0][t] - d[2][t], d[1][t] + d[2][t], d[2][t] - d[1][t], d[1][t] - d[3][t]) for t in range(n)]
            z = [[[], [], []], [[], [], []]]
            for b in range(3):
                for t in range(n):
                    m0, m1, m2, m3 = (T[t][k] * wv[k * 3 + b] for k in range(4))
                    z[0][b].append(m0 + m1 + m2)
                    z[1][b].append(m1 - m2 - m3)
            return z

        def shift_sum(z1, Rr, Ll, t):
            lane = lax.broadcasted_iota(jnp.int32, (8, 128), 1)
            lt = jnp.where(lane == 0, Rr[t - 1] if t > 0 else 0.0, Rr[t])
            rt = jnp.where(lane == 127, Ll[t + 1] if t < NT - 1 else 0.0, Ll[t])
            return z1[t] + lt + rt

        def fold4(v):
            s = lax.broadcasted_iota(jnp.int32, (8, 128), 0)
            m4 = s < 4
            m2 = (s & 2) == 0
            a = jnp.where(m4, v[0], v[1]) + pltpu.roll(jnp.where(m4, v[1], v[0]), 4, 0)
            b = jnp.where(m4, v[2], v[3]) + pltpu.roll(jnp.where(m4, v[3], v[2]), 4, 0)
            w = jnp.where(m2, a + pltpu.roll(a, 6, 0), b + pltpu.roll(b, 2, 0))
            return w + pltpu.roll(w, 7, 0)

        def rstd4(s1, s2):
            m = fold4(s1) * (1.0 / C)
            q = fold4(s2) * (1.0 / C)
            return lax.rsqrt(jnp.maximum(q - m * m, 0.0) + _EPS)

        def pick(rs, t):
            sl = (0, 4, 2, 6)[t]
            return rs[sl:sl + 1, :]

        def aug(hn):
            n = hn.shape[1]
            r8 = lax.broadcasted_iota(jnp.int32, (8, n), 0)
            ones = jnp.where(r8 < 2, 1.0, 0.0).astype(F32)
            return jnp.concatenate([hn, ones, jnp.zeros((128 - C - 8, n), F32)], axis=0)

        zs[0] = 0
        zs[1] = 0
        zs[2] = 0
        LX = LA - U
        head = pltpu.make_async_copy(x_hbm.at[pl.ds(0, U)], xbuf.at[NXB - 1], xsem.at[NXB - 1])
        head2 = pltpu.make_async_copy(x_hbm.at[pl.ds(U, LX)], obuf.at[NOB - 1, pl.ds(0, LX)], osem.at[NOB - 1])
        head.start()
        head2.start()
        xchunk(0).start()
        xchunk(1).start()
        rows = [dw_ref[a, b:b + 1, :].astype(F32) for a in range(3) for b in range(3)]
        plain = list(rows)
        if WINO:
            g0, g1, g2 = rows[0:3], rows[3:6], rows[6:9]
            rows = g0 + [(a + b + c) * 0.5 for a, b, c in zip(g0, g1, g2)] + [(a - b + c) * 0.5 for a, b, c in zip(g0, g1, g2)] + g2
        rows.append(b2_ref[...].astype(F32))
        rows.append(g_ref[...].astype(F32))
        p = jnp.concatenate(rows + [jnp.zeros((128 - len(rows), C), F32)], axis=0)
        p = jnp.concatenate([p, jnp.zeros((128, 128 - C), F32)], axis=1)
        pt = p.T
        for k in range(NWT):
            xf[RING + k // 4, :, (k % 4) * 128:(k % 4) * 128 + 128] = jnp.broadcast_to(pt[:C, k:k + 1], (C, 128))
        gcol = pt[:C, NWT + 1:NWT + 2]
        xf[RING + 3, :, 0:128] = jnp.broadcast_to(pt[:C, NWT:NWT + 1] * gcol, (C, 128))
        w2f = (w2t_ref[...].astype(F32) * (gcol * (0.5 / _A))).astype(BF16)
        for k in range(NK):
            w2s[k] = pltpu.bitcast(w2f[:, k * 128:(k + 1) * 128], U32)
        w1 = w1_ref[...].astype(F32)
        w1c = (w1 - jnp.mean(w1, axis=0, keepdims=True)) * _A
        b1 = b1_ref[...].astype(F32) * _A
        b1h = b1.astype(BF16).astype(F32)
        b1l = b1 - b1h
        r8 = lax.broadcasted_iota(jnp.int32, (8, E), 0)
        tail = jnp.where(r8 == 0, b1h, jnp.where(r8 == 1, b1l, 0.0))
        waug = jnp.concatenate([w1c, tail, jnp.zeros((128 - C - 8, E), F32)], axis=0)
        wt = waug.T
        wt = jnp.concatenate([wt[kk * 128 + j * 8:kk * 128 + j * 8 + 8] for kk in range(NK) for j in reversed(range(16))], axis=0)
        w1s[0] = pltpu.bitcast(wt.astype(BF16), U32)
        xf[0] = jnp.zeros((C, W), F32)
        xf[1] = jnp.zeros((C, W), F32)
        gs[...] = jnp.zeros(gs.shape, F32)
        head.wait()
        head2.wait()
        PR = o.get('pr', 4)
        for r in range(LX):
            xf[r + 2] = xbuf[NXB - 1, r].astype(F32)
        for r in range(LX - 1, LA):
            pass

        def cp(r, _):
            xf[r + 2] = xbuf[NXB - 1, r].astype(F32)
            return 0
        lax.fori_loop(LX, U, cp, 0)
        for r in range(LX):
            xf[U + r + 2] = obuf[NOB - 1, r].astype(F32)

        def cv(rr, _):
            r = rr * PR
            s1 = [[0.0] * NT for _ in range(PR)]
            s2 = [[0.0] * NT for _ in range(PR)]
            for cg in range(NCG):
                cs = slice(cg * 8, cg * 8 + 8)
                xs = [xf[r + 1 + q, cs, :] for q in range(PR + 2)]
                for q in range(PR):
                    y = conv_piece(cg, xs[q], xs[q + 1], xs[q + 2], xf, wino=False)
                    ya[r + q, cs, :] = jnp.concatenate(y, axis=1)
                    s1[q] = [a + b for a, b in zip(s1[q], y)]
                    s2[q] = [a + b * b for a, b in zip(s2[q], y)]
            for q in range(PR):
                v = r + q
                ya[U, pl.ds(pl.multiple_of((v % 12) * 8, 8), 8), pl.ds(pl.multiple_of(128 + 128 * (v // 12), 128), 128)] = rstd4(s1[q], s2[q])
            return 0
        lax.fori_loop(0, U // PR, cv, 0)

        mm = lambda a, b: lax.dot_general(a, b, (((1,), (0,)), ((), ())), preferred_element_type=F32)

        def rev(g, kk):
            return jnp.concatenate([g[kk * 128 + j * 8:kk * 128 + j * 8 + 8] for j in reversed(range(16))], axis=0)

        def block(k, ycur, ynxt):
            r0 = k * U
            z0 = zs[0]
            z1 = zs[1]
            z2 = zs[2]
            src = xbuf.at[k % NXB]
            ocur = obuf.at[k % NOB]
            onxt = obuf.at[(k + 1) % NOB]
            wd = xf.at[pl.ds(z0, RING + 4)]
            ybd = ycur.at[pl.ds(z0, U + 1)]
            rbase = (k % 4) * U + 1

            def ring(r):
                return (rbase + r + 1) & (RING - 1)

            ev = []
            st = dict(n=0, s1=None, s2=None, z=None, up=LA, nup=0, out=[])
            evr = []
            ev2 = []
            vals = {}

            def token(T, wide=False, side=False):
                c = [e for e in ev if e[0] <= T + 1e-6]
                if side:
                    late = max([e[0] for e in c], default=-99)
                    c += [e for e in ev2 if late + 1.0 < e[0] <= T + 1e-6]
                if not c:
                    return None
                _, a, j = max(c, key=lambda e: e[0])
                return a[j * 8:j * 8 + 8, 0:256].astype(BF16) if wide else a[j * 8:j * 8 + 8, 0:128]

            def xtok(v, T=None):
                c = [e for e in evr if T is not None and T - o.get('rwin', 2) <= e[0] <= T]
                if c:
                    for e in c:
                        xf[RING + 3 + z2, 0:8, 384:512] = e[1]
                        evr.remove(e)
                    if not o.get('both', 0):
                        return
                xf[RING + 3 + z2, 0:8, 384:512] = v

            def conv_next(v_, T=None):
                v, n = divmod(st['n'], NCG)
                if v >= U:
                    return
                if v_ is not None:
                    xtok(v_, T)
                if WINO:
                    v, n, part = 2 * (st['n'] // 24), (st['n'] % 24) // 2, st['n'] % 2
                    assert v + U + 2 < st['up'], (v, st['up'])
                    cs = slice(n * 8, n * 8 + 8)
                    ts = slice(part * HW, part * HW + HW)
                    z = wino_front(n, [xf[ring(v + U - 1 + q), cs, ts] for q in range(4)], wd)
                    st['z'] = [None, [None, None, z[1][1][1]]]
                    zz_ = st['zk'] if part else [[[], [], []], [[], [], []]]
                    for q in range(2):
                        zz_[q][0] += [pltpu.roll(a, 1, 1) for a in z[q][0]]
                        zz_[q][1] += z[q][1]
                        zz_[q][2] += [pltpu.roll(a, 127, 1) for a in z[q][2]]
                    st['zk'] = zz_
                    if part == 0:
                        st['y0'] = [shift_sum(zz_[q][1], zz_[q][0], zz_[q][2], 0) for q in range(2)]
                    else:
                        for q in range(2):
                            y = [st['y0'][q]] + [shift_sum(zz_[q][1], zz_[q][0], zz_[q][2], t) for t in range(1, NT)]
                            finish(v + q, n, y, q)
                else:
                    assert v + U + 1 < st['up'], (v, st['up'])
                    cs = slice(n * 8, n * 8 + 8)
                    y, st['z'] = conv_piece(n, xf[ring(v + U - 1), cs, :], xf[ring(v + U), cs, :], xf[ring(v + U + 1), cs, :], wd, True)
                    finish(v, n, y, 0)
                    if T is not None:
                        ev2.append((T + o.get('zdt', 2), st['z'][1][3], 0))
                        ev2.append((T + o.get('ydt', 5), y[3], 0))
                st['n'] += 1

            def finish(v, n, y, q):
                ynxt[v, n * 8:n * 8 + 8, :] = jnp.concatenate(y, axis=1)
                if n == 0:
                    st['s1', q], st['s2', q] = y, [b * b for b in y]
                else:
                    st['s1', q] = [a + b for a, b in zip(st['s1', q], y)]
                    st['s2', q] = [a + b * b for a, b in zip(st['s2', q], y)]
                if n == NCG - 1:
                    ynxt[U, (v % 12) * 8:(v % 12) * 8 + 8, 128 + 128 * (v // 12):256 + 128 * (v // 12)] = rstd4(st['s1', q], st['s2', q])

            def run(T, kind, u, h, n):
                if kind == 'c':
                    v = token(T)
                    conv_next(v if v is not None or st['z'] is None else st['z'][1][2], T)
                elif kind == 'z':
                    conv_next(None if st['z'] is None else st['z'][1][2])
                elif kind == 'up':
                    c = [e for e in st['out'] if T - o.get('uwin', 0) <= e[0] <= T]
                    v = c[-1][1] if c else token(T, True)
                    if v is not None:
                        xbuf[NXB + z1, 0, 0:8, 0:256] = v
                    cs = slice(n * (C // NUP), (n + 1) * (C // NUP))
                    xf[ring(st['up']), cs, :] = src[u, cs, :].astype(F32)
                    st['nup'] += 1
                    if n == NUP - 1:
                        st['up'] += 1
                elif kind == 'ld':
                    v = token(T)
                    if v is not None:
                        ycur[U + z1, 0:8, 0:128] = v
                    if ('rs', u) not in vals:
                        vals['rs', u] = ybd[U, (u % 12) * 8:(u % 12) * 8 + 8, 128 + 128 * (u // 12):256 + 128 * (u // 12)]
                    t = 2 * h + n
                    vals['h', u, t] = ybd[u, :, t * 128:(t + 1) * 128] * pick(vals['rs', u], t)
                elif kind == 'w1':
                    v = token(T, side=o.get('side', 0))
                    if v is not None:
                        w1s[1 + z1, 0:8, :] = pltpu.bitcast(v, U32)
                    a0, a1 = n
                    vals.setdefault(('w1', u, h), []).append(w1s[z0, a0 * 8:a1 * 8, :])
                elif kind == 'w2':
                    v = token(T)
                    if v is not None:
                        w2s[NK + z1, 0:8, :] = pltpu.bitcast(v, U32)
                    vals['w2', u, h, n] = w2s[n + z0]
                elif kind == 'gl':
                    v = token(T)
                    if v is not None:
                        gs[E + z1 * 8:E + z1 * 8 + 8, 0:128] = v
                    vals['g', u, h, n] = gs[pl.ds(pl.multiple_of(z0 * 8 + n * 128, 8), 128), :]
                elif kind == 'gp':
                    m = (n // 16) * 16 + 15 - n % 16
                    gs[m * 8:m * 8 + 8, :] = vals['graw'][n * 8:n * 8 + 8, :]
                elif kind == 'pk':
                    kk, q = n
                    nr = C // NRP
                    rs8 = slice(q * nr, q * nr + nr)
                    P = vals['P', u, h]
                    if MODE == 3:
                        accx[2 * h + kk + z1, rs8, :] = P[kk][rs8]
                    elif MODE == 5:
                        if kk == 0:
                            accx[2 * h + z1, rs8, :] = P[0][rs8]
                    elif MODE == 0:
                        pass
                    elif kk == 1:
                        accx[2 * h + z1, rs8, :] = P[0][rs8] + P[1][rs8]
                elif kind == 'r':
                    v = token(T)
                    if v is not None:
                        if not o.get('noxf', 0):
                            xtok(v)
                        if MODE != 0:
                            accx[4 + z1, 0:8, 0:128] = v
                    nr = C // NRP
                    rs8 = slice(n * nr, n * nr + nr)
                    hs = slice(h * HW, h * HW + HW)
                    gbv = wtap(wd, 12, rs8)
                    res = xf[ring(u), rs8, hs] + jnp.concatenate([gbv, gbv], axis=1)
                    P = vals['P', u, h]
                    if MODE == 0:
                        a = (P[0][rs8] + P[1][rs8]) + res
                    elif MODE == 5:
                        a = (accx[2 * h + z0, rs8, :] + res) + P[1][rs8]
                    else:
                        a = accx[2 * h + z0, rs8, :] + res
                    if MODE == 3:
                        a = a + accx[2 * h + 1 + z0, rs8, :]
                    outf = a + vals['P', u, h][2][rs8]
                    out = outf.astype(o_hbm.dtype)
                    st['out'].append((T, out[nr - 8:nr, :]))
                    if o.get('rtok', 0):
                        for t_ in range(o['rtok']):
                            evr.append((T + 0.02, outf[nr - 8 * (1 + t_ // 2):, 128 * (1 - t_ % 2):][0:8, 0:128]))
                    if u + 1 < U:
                        ocur[u + 1, rs8, hs] = out
                    else:
                        onxt[0, rs8, hs] = out

            S0 = ((0.0, 0.0), (18.0, 0.0))
            items = []
            w1items = {}
            add = lambda T, kind, u, h, n: items.append((T, len(items), kind, u, h, n))
            for e in range(o.get('early', 0)):
                add(-20 + e, 'z', 0, 0, 0)
            m2start = lambda u, h: 42 * u + (24 if h == 0 else 42)
            for u in range(-1, U):
                if u >= 0:
                    for tau in o['c']:
                        add(42 * u + tau, 'c', u, 0, 0)
                    for n in range(NUP):
                        add(42 * u + o['up'][n], 'up', u, 0, n)
                for h in range(2):
                    if u >= 0:
                        m1 = 42 * u + S0[h][0]
                        for n in range(2):
                            add(m1 - o['ld'][n], 'ld', u, h, n)
                        a0 = 0
                        for nst, dt in (o['w1c'] if h == 0 else o.get('w1b', o['w1c'])):
                            w1items.setdefault((u, h), []).append((m1 + a0 - dt, 'w1', u, h, (a0, a0 + nst)))
                            a0 += nst
                    if (u == U - 1 and h == 1):
                        for j in range(48):
                            add(42 * u + 27 + j / 2, 'gp', u, h, j)
                        continue
                    if (u == -1 and h == 0):
                        continue
                    m2 = m2start(u, h)
                    w = 6.0 / NRP
                    for kk in range(NK):
                        add(m2 + 6 * kk - o['w2dt'], 'w2', u, h, kk)
                        if u == -1:
                            add(m2 + 6 * kk - 6, 'gl', u, h, kk)
                        if kk < 2:
                            for q in range(NRP):
                                add(m2 + 8 + 6 * kk + (q + 1) * w - 0.5, 'pk', u, h, (kk, q))
                    for q in range(NRP):
                        add(m2 + 20 + q * w + o['roff'], 'r', u, h, q)
            items.sort()
            ptr = [0]

            def flush(pred):
                last = max([i_ for i_, it in enumerate(items) if pred(it)], default=-1)
                while ptr[0] <= last:
                    T, _, kind, u, h, n = items[ptr[0]]
                    run(T, kind, u, h, n)
                    ptr[0] += 1

            def mat1(u, h):
                flush(lambda it: (it[2] == 'ld' and it[3] == u and it[4] == h) or (o.get('side', 0) and it[2] == 'c' and it[0] < 42 * u + S0[h][0] + (8 if h == 0 else 5)))
                for it in w1items[u, h]:
                    run(*it)
                lhs = jnp.concatenate(vals['w1', u, h], axis=0)
                rhs = jnp.concatenate([vals['h', u, 2 * h], vals['h', u, 2 * h + 1]], axis=1)
                zz = mm(pltpu.bitcast(lhs, BF16), aug(rhs))
                tt = zz * (zz * zz + _C0)
                g = zz * jnp.tanh(tt) + zz
                vals['graw'] = g
                for kk in range(NK):
                    vals['g', u, h, kk] = rev(g, kk)
                ev.extend((42 * u + S0[h][0] + 9 + j / 2, g, j) for j in range(48))

            def mat2(u, h):
                flush(lambda it: it[2] in ('w2', 'gl') and it[3] == u and it[4] == h)
                P = [mm(pltpu.bitcast(vals['w2', u, h, kk], BF16), vals['g', u, h, kk]) for kk in range(NK)]
                vals['P', u, h] = P
                ev.extend((m2start(u, h) + 8 + 6 * kk + j / 2 + 0.01, P[kk], j) for kk in range(NK) for j in range(12))

            for u in range(U):
                mat1(u, 0)
                mat2(u - 1, 1)
                mat1(u, 1)
                mat2(u, 0)
            flush(lambda it: True)
            assert st['n'] == U * NCG and st['up'] == LA + U, st

        def body(k, _):
            pl.when(k < KP)(lambda: xchunk(k).wait())

            @pl.when(k == KP)
            def _():
                if NP:
                    xpart().wait()
                xbuf[KP % NXB, NP] = jnp.zeros((C, W), BF16)

            pl.when(k + 2 < KP)(lambda: xchunk(k + 2).start())
            if NP:
                pl.when(k + 2 == KP)(lambda: xpart().start())
            pl.when(k % 2 == 0)(lambda: block(k, ya, yb))
            pl.when(k % 2 == 1)(lambda: block(k, yb, ya))
            pl.when(k == 2)(lambda: ofirst.wait())
            pl.when(k > 2)(lambda: ochunk(k - 2).wait())
            pl.when(k == 0)(lambda: ofirst.start())
            pl.when(k > 0)(lambda: ochunk(k).start())
            return 0

        lax.fori_loop(0, NBLK, body, 0)

        acc = xf[(H - 1 + 2) % RING, :, HW:] + jnp.concatenate([wtap(xf, 12, slice(0, C))] * 2, axis=1)
        for kk in range(NK):
            acc = acc + mm(pltpu.bitcast(w2s[kk], BF16), gs[kk * 128:(kk + 1) * 128, :])
        obuf[NBLK % NOB, 0, :, HW:] = acc.astype(o_hbm.dtype)
        olast.start()
        ochunk(NBLK - 2).wait()
        ochunk(NBLK - 1).wait()
        olast.wait()

    return kernel, RING


_U = 8
_SCHED = {'c': (2.58, 6.0, 9.42, 12.83, 16.25, 19.67, 23.08, 27.5, 30.92, 34.33, 37.75, 41.17), 'up': (4.0, 6.0, 8.0, 10.0, 12.0, 14.0), 'ld': (7.5, 6.0), 'w1c': ((24, 3),), 'w2dt': 4, 'roff': -1, 'nrp': 4, 'mode': 0, 'early': 1, 'noxf': 1, 'wino': 0, 'nodma': 0, 'side': 0, 'zdt': 2, 'ydt': 5, 'rtok': 0, 'rwin': 2, 'uwin': 0, 'both': 0, 'w1b': ((24, 3),)}


@jax.jit
def pallas_standalone__modern_conv_block_convnext__vision_kernel(x, dw, w1, b1, w2, b2, gamma):
    U, O, FLAGS = _U, _SCHED, ()
    B, H, W, C = x.shape
    E = w1.shape[1]
    xt = jnp.transpose(x[0], (0, 2, 1))
    args = (dw, w1, b1.reshape(1, E), w2.T, b2.reshape(1, C), gamma.reshape(1, C))
    kern, RING = _make(H, C, W, E, U, dict(O))
    vm = pl.BlockSpec(memory_space=pltpu.VMEM)
    out = pl.pallas_call(
        kern,
        in_specs=[pl.BlockSpec(memory_space=pl.ANY)] + [vm for a in args],
        out_specs=pl.BlockSpec(memory_space=pl.ANY),
        out_shape=jax.ShapeDtypeStruct((H, C, W), x.dtype),
        scratch_shapes=[
            pltpu.VMEM((5, U, C, W), BF16),
            pltpu.VMEM((4, U, C, W), BF16),
            pltpu.SemaphoreType.DMA((4,)),
            pltpu.SemaphoreType.DMA((4,)),
            pltpu.VMEM((2, E // 2, 128), U32),
            pltpu.VMEM((E // 128 + 1, C // 2, 128), U32),
            pltpu.VMEM((RING + 4, C, W), F32),
            pltpu.VMEM((U + 1, C, W), F32),
            pltpu.VMEM((U + 1, C, W), F32),
            pltpu.VMEM((5, C, W // 2), F32),
            pltpu.VMEM((E + 8, W // 2), F32),
            pltpu.SMEM((3,), jnp.int32),
        ],
        compiler_params=pltpu.CompilerParams(vmem_limit_bytes=96 * 1024 * 1024, flags=dict(FLAGS), disable_bounds_checks=bool(dict(O).get('nobc', 1))),
    )(xt, *args)
    return jnp.transpose(out, (0, 2, 1))[None]
```

```python
import functools
import jax
import jax.numpy as jnp
from jax import lax
import jax.experimental.pallas as pl
import jax.experimental.pallas.tpu as pltpu
import numpy as np

_K0 = float(np.sqrt(2.0 / np.pi))
_K1 = _K0 * 0.044715
_A = _K1 ** (1.0 / 3.0)
_C0 = _K0 / _A
_EPS = 1e-5
F32 = jnp.float32
BF16 = jnp.bfloat16
U32 = jnp.uint32


def _make(H, C, W, E, U, o):
    NBLK = H // U
    NT = W // 128
    NCG = C // 8
    NK = E // 128
    NUP = 6
    WINO = 0
    NWT = 12 if WINO else 9
    XL = o.get('xl', 1) + WINO
    LA = U + 2 + XL
    RING = 4 * U
    NXB = 4
    NOB = 4
    HW = W // 2
    NRP = o.get('nrp', 4)
    MODE = o.get('mode', 3)
    assert NBLK % 2 == 0

    def kernel(x_hbm, dw_ref, w1_ref, b1_ref, w2t_ref, b2_ref, g_ref, o_hbm,
               io, xsem, osem, w1s, w2s, xf, ya, yb, accx, gs, zs):

        xbuf = io.at[pl.ds(0, 5)]
        obuf = io.at[pl.ds(5, 4)]

        def xchunk(k):
            s_ = k % NXB
            return pltpu.make_async_copy(x_hbm.at[pl.ds(k * U + LA, U)], xbuf.at[s_], xsem.at[s_])

        KP = (H - LA) // U
        NP = H - LA - KP * U

        def xpart():
            return pltpu.make_async_copy(x_hbm.at[pl.ds(H - NP, NP)], xbuf.at[KP % NXB, pl.ds(0, NP)], xsem.at[KP % NXB])

        def ochunk(k):
            s_ = k % NOB
            return pltpu.make_async_copy(obuf.at[s_], o_hbm.at[pl.ds(k * U - 1, U)], osem.at[s_])

        ofirst = pltpu.make_async_copy(obuf.at[0, pl.ds(1, U - 1)], o_hbm.at[pl.ds(0, U - 1)], osem.at[0])
        olast = pltpu.make_async_copy(obuf.at[NBLK % NOB, pl.ds(0, 1)], o_hbm.at[pl.ds(H - 1, 1)], osem.at[NBLK % NOB])

        def tiles(v):
            return [v[:, t * 128:(t + 1) * 128] for t in range(NT)]

        def wtap(ref, k, cs):
            return ref[RING + k // 4, cs, (k % 4) * 128:(k % 4) * 128 + 128]

        def conv_piece(cg, x0, x1, x2, wref, want_z=False, wino=False):
            lane = lax.broadcasted_iota(jnp.int32, (8, 128), 1)
            cs = slice(cg * 8, cg * 8 + 8)
            wv = [wtap(wref, k, cs) for k in range(9)]
            x0, x1, x2 = tiles(x0), tiles(x1), tiles(x2)
            z = [[x0[t] * wv[b] + x1[t] * wv[3 + b] + x2[t] * wv[6 + b] for t in range(NT)] for b in range(3)]
            if o.get('casc', 0):
                L1 = [pltpu.roll(v, 127, 1) for v in z[1]]
                L2 = [pltpu.roll(v, 127, 1) for v in z[2]]
                bb = [z[0][t] + jnp.where(lane == 127, L1[t + 1] if t < NT - 1 else 0.0, L1[t]) for t in range(NT)]
                Rb = [pltpu.roll(v, 1, 1) for v in bb]
                out = [jnp.where(lane == 0, Rb[t - 1] if t > 0 else z[1][0], Rb[t])
                       + jnp.where(lane == 127, L2[t + 1] if t < NT - 1 else 0.0, L2[t]) for t in range(NT)]
            else:
                Rr = [pltpu.roll(v, 1, 1) for v in z[0]]
                Ll = [pltpu.roll(v, 127, 1) for v in z[2]]
                out = []
                for t in range(NT):
                    lt = jnp.where(lane == 0, Rr[t - 1] if t > 0 else 0.0, Rr[t])
                    rt = jnp.where(lane == 127, Ll[t + 1] if t < NT - 1 else 0.0, Ll[t])
                    out.append(z[1][t] + lt + rt)
            return (out, z) if want_z else out

        def direct_front(cg, d, wref):
            cs = slice(cg * 8, cg * 8 + 8)
            wv = [wtap(wref, k, cs) for k in range(9)]
            n = d[0].shape[1] // 128
            d = [[v[:, t * 128:(t + 1) * 128] for t in range(n)] for v in d]
            return [[d[0][t] * wv[b] + d[1][t] * wv[3 + b] + d[2][t] * wv[6 + b] for t in range(n)] for b in range(3)]

        def wino_front(cg, d, wref):
            cs = slice(cg * 8, cg * 8 + 8)
            wv = [wtap(wref, k, cs) for k in range(12)]
            n = d[0].shape[1] // 128
            d = [[v[:, t * 128:(t + 1) * 128] for t in range(n)] for v in d]
            T = [(d[0][t] - d[2][t], d[1][t] + d[2][t], d[2][t] - d[1][t], d[1][t] - d[3][t]) for t in range(n)]
            z = [[[], [], []], [[], [], []]]
            for b in range(3):
                for t in range(n):
                    m0, m1, m2, m3 = (T[t][k] * wv[k * 3 + b] for k in range(4))
                    z[0][b].append(m0 + m1 + m2)
                    z[1][b].append(m1 - m2 - m3)
            return z

        def shift_sum(z1, Rr, Ll, t):
            lane = lax.broadcasted_iota(jnp.int32, (8, 128), 1)
            lt = jnp.where(lane == 0, Rr[t - 1] if t > 0 else 0.0, Rr[t])
            rt = jnp.where(lane == 127, Ll[t + 1] if t < NT - 1 else 0.0, Ll[t])
            return z1[t] + lt + rt

        def fold4(v):
            s = lax.broadcasted_iota(jnp.int32, (8, 128), 0)
            m4 = s < 4
            m2 = (s & 2) == 0
            a = jnp.where(m4, v[0], v[1]) + pltpu.roll(jnp.where(m4, v[1], v[0]), 4, 0)
            b = jnp.where(m4, v[2], v[3]) + pltpu.roll(jnp.where(m4, v[3], v[2]), 4, 0)
            w = jnp.where(m2, a + pltpu.roll(a, 6, 0), b + pltpu.roll(b, 2, 0))
            return w + pltpu.roll(w, 7, 0)

        def rstd4(s1, s2):
            m = fold4(s1) * (1.0 / C)
            q = fold4(s2) * (1.0 / C)
            return lax.rsqrt(jnp.maximum(q - m * m, 0.0) + _EPS)

        def pick(rs, t):
            sl = (0, 4, 2, 6)[t]
            return rs[sl:sl + 1, :]

        def aug(hn):
            n = hn.shape[1]
            r8 = lax.broadcasted_iota(jnp.int32, (8, n), 0)
            ones = jnp.where(r8 < 2, 1.0, 0.0).astype(F32)
            return jnp.concatenate([hn, ones, jnp.zeros((128 - C - 8, n), F32)], axis=0)

        zs[0] = 0
        zs[1] = 0
        zs[2] = 0
        LX = LA - U
        head = pltpu.make_async_copy(x_hbm.at[pl.ds(0, U)], xbuf.at[NXB - 1], xsem.at[NXB - 1])
        head2 = pltpu.make_async_copy(x_hbm.at[pl.ds(U, LX)], obuf.at[NOB - 1, pl.ds(0, LX)], osem.at[NOB - 1])
        head.start()
        head2.start()
        xchunk(0).start()
        xchunk(1).start()
        rows = [dw_ref[a, b:b + 1, :].astype(F32) for a in range(3) for b in range(3)]
        plain = list(rows)
        if WINO:
            g0, g1, g2 = rows[0:3], rows[3:6], rows[6:9]
            rows = g0 + [(a + b + c) * 0.5 for a, b, c in zip(g0, g1, g2)] + [(a - b + c) * 0.5 for a, b, c in zip(g0, g1, g2)] + g2
        rows.append(b2_ref[...].astype(F32))
        rows.append(g_ref[...].astype(F32))
        p = jnp.concatenate(rows + [jnp.zeros((128 - len(rows), C), F32)], axis=0)
        p = jnp.concatenate([p, jnp.zeros((128, 128 - C), F32)], axis=1)
        pt = p.T
        for k in range(NWT):
            xf[RING + k // 4, :, (k % 4) * 128:(k % 4) * 128 + 128] = jnp.broadcast_to(pt[:C, k:k + 1], (C, 128))
        gcol = pt[:C, NWT + 1:NWT + 2]
        xf[RING + 3, :, 0:128] = jnp.broadcast_to(pt[:C, NWT:NWT + 1] * gcol, (C, 128))
        w2f = (w2t_ref[...].astype(F32) * (gcol * (0.5 / _A))).astype(BF16)
        for k in range(NK):
            w2s[k] = pltpu.bitcast(w2f[:, k * 128:(k + 1) * 128], U32)
        w1 = w1_ref[...].astype(F32)
        w1c = (w1 - jnp.mean(w1, axis=0, keepdims=True)) * _A
        b1 = b1_ref[...].astype(F32) * _A
        b1h = b1.astype(BF16).astype(F32)
        b1l = b1 - b1h
        r8 = lax.broadcasted_iota(jnp.int32, (8, E), 0)
        tail = jnp.where(r8 == 0, b1h, jnp.where(r8 == 1, b1l, 0.0))
        waug = jnp.concatenate([w1c, tail, jnp.zeros((128 - C - 8, E), F32)], axis=0)
        wt = waug.T
        wt = jnp.concatenate([wt[kk * 128 + j * 8:kk * 128 + j * 8 + 8] for kk in range(NK) for j in reversed(range(16))], axis=0)
        w1s[0] = pltpu.bitcast(wt.astype(BF16), U32)
        xf[0] = jnp.zeros((C, W), F32)
        xf[1] = jnp.zeros((C, W), F32)
        gs[...] = jnp.zeros(gs.shape, F32)
        head.wait()
        head2.wait()
        PR = o.get('pr', 4)
        for r in range(LX):
            xf[r + 2] = xbuf[NXB - 1, r].astype(F32)
        for r in range(LX - 1, LA):
            pass

        def cp(r, _):
            xf[r + 2] = xbuf[NXB - 1, r].astype(F32)
            return 0
        lax.fori_loop(LX, U, cp, 0)
        for r in range(LX):
            xf[U + r + 2] = obuf[NOB - 1, r].astype(F32)

        def cv(rr, _):
            r = rr * PR
            s1 = [[0.0] * NT for _ in range(PR)]
            s2 = [[0.0] * NT for _ in range(PR)]
            for cg in range(NCG):
                cs = slice(cg * 8, cg * 8 + 8)
                xs = [xf[r + 1 + q, cs, :] for q in range(PR + 2)]
                for q in range(PR):
                    y = conv_piece(cg, xs[q], xs[q + 1], xs[q + 2], xf, wino=False)
                    ya[r + q, cs, :] = jnp.concatenate(y, axis=1)
                    s1[q] = [a + b for a, b in zip(s1[q], y)]
                    s2[q] = [a + b * b for a, b in zip(s2[q], y)]
            for q in range(PR):
                v = r + q
                ya[U, pl.ds(pl.multiple_of((v % 12) * 8, 8), 8), pl.ds(pl.multiple_of(128 + 128 * (v // 12), 128), 128)] = rstd4(s1[q], s2[q])
            return 0
        lax.fori_loop(0, U // PR, cv, 0)

        mm = lambda a, b: lax.dot_general(a, b, (((1,), (0,)), ((), ())), preferred_element_type=F32)

        def rev(g, kk):
            return jnp.concatenate([g[kk * 128 + j * 8:kk * 128 + j * 8 + 8] for j in reversed(range(16))], axis=0)

        def block(k, ycur, ynxt):
            r0 = k * U
            z0 = zs[0]
            z1 = zs[1]
            z2 = zs[2]
            src = xbuf.at[k % NXB]
            ocur = obuf.at[k % NOB]
            onxt = obuf.at[(k + 1) % NOB]
            wd = xf.at[pl.ds(z0, RING + 4)]
            ybd = ycur.at[pl.ds(z0, U + 1)]
            rbase = (k % 4) * U + 1

            def ring(r):
                return (rbase + r + 1) & (RING - 1)

            ev = []
            st = dict(n=0, s1=None, s2=None, z=None, up=LA, nup=0, out=[])
            evr = []
            ev2 = []
            vals = {}

            def token(T, wide=False, side=False):
                c = [e for e in ev if e[0] <= T + 1e-6]
                if side:
                    late = max([e[0] for e in c], default=-99)
                    c += [e for e in ev2 if late + 1.0 < e[0] <= T + 1e-6]
                if not c:
                    return None
                _, a, j = max(c, key=lambda e: e[0])
                return a[j * 8:j * 8 + 8, 0:256].astype(BF16) if wide else a[j * 8:j * 8 + 8, 0:128]

            def xtok(v, T=None):
                c = [e for e in evr if T is not None and T - o.get('rwin', 2) <= e[0] <= T]
                if c:
                    for e in c:
                        xf[RING + 3 + z2, 0:8, 384:512] = e[1]
                        evr.remove(e)
                    if not o.get('both', 0):
                        return
                xf[RING + 3 + z2, 0:8, 384:512] = v

            def conv_next(v_, T=None):
                v, n = divmod(st['n'], NCG)
                if st['n'] >= U * NCG * (1 + o.get('half', 0)):
                    return
                if v_ is not None:
                    xtok(v_, T)
                if o.get('half', 0):
                    v, n, part = st['n'] // 24, (st['n'] % 24) // 2, st['n'] % 2
                    assert v + U + 1 < st['up'], (v, st['up'])
                    cs = slice(n * 8, n * 8 + 8)
                    ts = slice(part * HW, part * HW + HW)
                    z = direct_front(n, [xf[ring(v + U - 1 + q), cs, ts] for q in range(3)], wd)
                    st['z'] = [None, [None, None, z[1][1]]]
                    zz_ = st['zk'] if part else [[], [], []]
                    zz_[0] += [pltpu.roll(a, 1, 1) for a in z[0]]
                    zz_[1] += z[1]
                    zz_[2] += [pltpu.roll(a, 127, 1) for a in z[2]]
                    st['zk'] = zz_
                    if part == 0:
                        st['y0'] = shift_sum(zz_[1], zz_[0], zz_[2], 0)
                    else:
                        finish(v, n, [st['y0']] + [shift_sum(zz_[1], zz_[0], zz_[2], t) for t in range(1, NT)], 0)
                elif WINO:
                    v, n, part = 2 * (st['n'] // 24), (st['n'] % 24) // 2, st['n'] % 2
                    assert v + U + 2 < st['up'], (v, st['up'])
                    cs = slice(n * 8, n * 8 + 8)
                    ts = slice(part * HW, part * HW + HW)
                    z = wino_front(n, [xf[ring(v + U - 1 + q), cs, ts] for q in range(4)], wd)
                    st['z'] = [None, [None, None, z[1][1][1]]]
                    zz_ = st['zk'] if part else [[[], [], []], [[], [], []]]
                    for q in range(2):
                        zz_[q][0] += [pltpu.roll(a, 1, 1) for a in z[q][0]]
                        zz_[q][1] += z[q][1]
                        zz_[q][2] += [pltpu.roll(a, 127, 1) for a in z[q][2]]
                    st['zk'] = zz_
                    if part == 0:
                        st['y0'] = [shift_sum(zz_[q][1], zz_[q][0], zz_[q][2], 0) for q in range(2)]
                    else:
                        for q in range(2):
                            y = [st['y0'][q]] + [shift_sum(zz_[q][1], zz_[q][0], zz_[q][2], t) for t in range(1, NT)]
                            finish(v + q, n, y, q)
                else:
                    assert v + U + 1 < st['up'], (v, st['up'])
                    cs = slice(n * 8, n * 8 + 8)
                    y, st['z'] = conv_piece(n, xf[ring(v + U - 1), cs, :], xf[ring(v + U), cs, :], xf[ring(v + U + 1), cs, :], wd, True)
                    finish(v, n, y, 0)
                    if T is not None:
                        ev2.append((T + o.get('zdt', 2), st['z'][1][3], 0))
                        ev2.append((T + o.get('ydt', 5), y[3], 0))
                st['n'] += 1

            def finish(v, n, y, q):
                ynxt[v, n * 8:n * 8 + 8, :] = jnp.concatenate(y, axis=1)
                if n == 0:
                    st['s1', q], st['s2', q] = y, [b * b for b in y]
                else:
                    if not o.get('hack4', 0): st['s1', q] = [a + b for a, b in zip(st['s1', q], y)]
                    if not o.get('hack3', 0): st['s2', q] = [a + b * b for a, b in zip(st['s2', q], y)]
                if n == NCG - 1:
                    ynxt[U, (v % 12) * 8:(v % 12) * 8 + 8, 128 + 128 * (v // 12):256 + 128 * (v // 12)] = rstd4(st['s1', q], st['s2', q])

            def run(T, kind, u, h, n):
                if kind == 'c':
                    v = token(T)
                    conv_next(v if v is not None or st['z'] is None else st['z'][1][2], T)
                elif kind == 'z':
                    conv_next(None if st['z'] is None else st['z'][1][2])
                elif kind == 'up':
                    c = [e for e in st['out'] if T - o.get('uwin', 0) <= e[0] <= T]
                    v = c[-1][1] if c else None if o.get('upfree', 0) and T > 8 else token(T, True)
                    if v is not None:
                        xbuf[NXB + z1, 0, 0:8, 0:256] = v
                    cs = slice(n * (C // NUP), (n + 1) * (C // NUP))
                    xf[ring(st['up']), cs, :] = src[u, cs, :].astype(F32)
                    st['nup'] += 1
                    if n == NUP - 1:
                        st['up'] += 1
                elif kind == 'ld':
                    v = token(T)
                    if v is not None:
                        ycur[U + z1, 0:8, 0:128] = v
                    if ('rs', u) not in vals:
                        vals['rs', u] = ybd[U, (u % 12) * 8:(u % 12) * 8 + 8, 128 + 128 * (u // 12):256 + 128 * (u // 12)]
                    t = 2 * h + n
                    vals['h', u, t] = ybd[u, :, t * 128:(t + 1) * 128] * pick(vals['rs', u], t)
                elif kind == 'w1':
                    v = token(T, side=o.get('side', 0))
                    if v is not None:
                        w1s[1 + z1, 0:8, :] = pltpu.bitcast(v, U32)
                    a0, a1 = n
                    vals.setdefault(('w1', u, h), []).append(w1s[z0, a0 * 8:a1 * 8, :])
                elif kind == 'w2':
                    v = token(T)
                    if v is not None:
                        w2s[NK + z1, 0:8, :] = pltpu.bitcast(v, U32)
                    vals['w2', u, h, n] = w2s[n + z0]
                elif kind == 'gl':
                    v = token(T)
                    if v is not None:
                        gs[E + z1 * 8:E + z1 * 8 + 8, 0:128] = v
                    vals['g', u, h, n] = gs[pl.ds(pl.multiple_of(z0 * 8 + n * 128, 8), 128), :]
                elif kind == 'gp':
                    m = (n // 16) * 16 + 15 - n % 16
                    gs[m * 8:m * 8 + 8, :] = vals['graw'][n * 8:n * 8 + 8, :]
                elif kind == 'pk':
                    kk, q = n
                    nr = C // NRP
                    rs8 = slice(q * nr, q * nr + nr)
                    P = vals['P', u, h]
                    if MODE == 3:
                        accx[2 * h + kk + z1, rs8, :] = P[kk][rs8]
                    elif MODE == 5:
                        if kk == 0:
                            accx[2 * h + z1, rs8, :] = P[0][rs8]
                    elif MODE == 0:
                        pass
                    elif kk == 1:
                        accx[2 * h + z1, rs8, :] = P[0][rs8] + P[1][rs8]
                elif kind == 'r':
                    v = token(T)
                    if v is not None:
                        if not o.get('noxf', 0):
                            xtok(v)
                        if MODE != 0:
                            accx[4 + z1, 0:8, 0:128] = v
                    nr = C // NRP
                    rs8 = slice(n * nr, n * nr + nr)
                    hs = slice(h * HW, h * HW + HW)
                    gbv = wtap(wd, 12, rs8)
                    res = xf[ring(u), rs8, hs] + jnp.concatenate([gbv, gbv], axis=1)
                    P = vals['P', u, h]
                    if MODE == 0:
                        a = (P[0][rs8] + P[1][rs8]) + res
                        if o.get('hack2', 0):
                            a = (P[0][rs8] + P[1][rs8])
                    elif MODE == 5:
                        a = (accx[2 * h + z0, rs8, :] + res) + P[1][rs8]
                    else:
                        a = accx[2 * h + z0, rs8, :] + res
                    if MODE == 3:
                        a = a + accx[2 * h + 1 + z0, rs8, :]
                    outf = a + vals['P', u, h][2][rs8]
                    out = outf.astype(o_hbm.dtype)
                    st['out'].append((T, out[nr - 8:nr, :]))
                    if o.get('rtok', 0):
                        for t_ in range(o['rtok']):
                            evr.append((T + 0.02, outf[nr - 8 * (1 + t_ // 2):, 128 * (1 - t_ % 2):][0:8, 0:128]))
                    if u + 1 < U:
                        ocur[u + 1, rs8, hs] = out
                    else:
                        onxt[0, rs8, hs] = out

            S0 = ((0.0, 0.0), (18.0, 0.0))
            items = []
            w1items = {}
            add = lambda T, kind, u, h, n: items.append((T, len(items), kind, u, h, n))
            for e in range(o.get('early', 0)):
                add(-20 + e, 'z', 0, 0, 0)
            m2start = lambda u, h: 42 * u + (24 if h == 0 else 42)
            for u in range(-1, U):
                if u >= 0:
                    for tau in o['c']:
                        add(42 * u + tau, 'c', u, 0, 0)
                    for n in range(NUP):
                        add(42 * u + o['up'][n], 'up', u, 0, n)
                for h in range(2):
                    if u >= 0:
                        m1 = 42 * u + S0[h][0]
                        for n in range(2):
                            add(m1 - (o['ld'] if h == 0 else o.get('ldb', o['ld']))[n], 'ld', u, h, n)
                        a0 = 0
                        for nst, dt in (o['w1c'] if h == 0 else o.get('w1b', o['w1c'])):
                            w1items.setdefault((u, h), []).append((m1 + a0 - dt, 'w1', u, h, (a0, a0 + nst)))
                            a0 += nst
                    if (u == U - 1 and h == 1):
                        for j in range(48):
                            add(42 * u + 27 + j / 2, 'gp', u, h, j)
                        continue
                    if (u == -1 and h == 0):
                        continue
                    m2 = m2start(u, h)
                    w = 6.0 / NRP
                    for kk in range(NK):
                        add(m2 + 6 * kk - (o['w2dt'][3 * h + kk] if isinstance(o['w2dt'], tuple) else o['w2dt']), 'w2', u, h, kk)
                        if u == -1:
                            add(m2 + 6 * kk - 6, 'gl', u, h, kk)
                        if kk < 2:
                            for q in range(NRP):
                                add(m2 + 8 + 6 * kk + (q + 1) * w - 0.5, 'pk', u, h, (kk, q))
                    for q in range(NRP):
                        add(m2 + 20 + q * w + (o['roff'][h] if isinstance(o['roff'], tuple) else o['roff']) + o.get('rgap', 0) * q, 'r', u, h, q)
            items.sort()
            ptr = [0]

            def flush(pred):
                last = max([i_ for i_, it in enumerate(items) if pred(it)], default=-1)
                while ptr[0] <= last:
                    T, _, kind, u, h, n = items[ptr[0]]
                    run(T, kind, u, h, n)
                    ptr[0] += 1

            def mat1(u, h):
                flush(lambda it: (it[2] == 'ld' and it[3] == u and it[4] == h) or (o.get('side', 0) and it[2] == 'c' and it[0] < 42 * u + S0[h][0] + (8 if h == 0 else 5)))
                for it in w1items[u, h]:
                    run(*it)
                lhs = jnp.concatenate(vals['w1', u, h], axis=0)
                if o.get('hack1', 0):
                    lhs = jnp.concatenate([lhs[0:48]] * 4, axis=0)
                rhs = jnp.concatenate([vals['h', u, 2 * h], vals['h', u, 2 * h + 1]], axis=1)
                zz = mm(pltpu.bitcast(lhs, BF16), aug(rhs))
                tt = zz * (zz * zz + _C0)
                g = zz * jnp.tanh(tt) + zz
                vals['graw'] = g
                for kk in range(NK):
                    vals['g', u, h, kk] = rev(g, kk)
                ev.extend((42 * u + S0[h][0] + 9 + j / 2, g, j) for j in range(48))

            def mat2(u, h):
                flush(lambda it: it[2] in ('w2', 'gl') and it[3] == u and it[4] == h)
                P = [mm(pltpu.bitcast(vals['w2', u, h, kk], BF16), vals['g', u, h, kk]) for kk in range(NK)]
                vals['P', u, h] = P
                ev.extend((m2start(u, h) + 8 + 6 * kk + j / 2 + 0.01, P[kk], j) for kk in range(NK) for j in range(12))

            for u in range(U):
                mat1(u, 0)
                mat2(u - 1, 1)
                mat1(u, 1)
                mat2(u, 0)
            flush(lambda it: True)
            assert st['n'] == U * NCG * (1 + o.get('half', 0)) and st['up'] == LA + U, st

        def body(k, _):
            pl.when(k < KP)(lambda: xchunk(k).wait())

            @pl.when(k == KP)
            def _():
                if NP:
                    xpart().wait()
                xbuf[KP % NXB, NP] = jnp.zeros((C, W), BF16)

            pl.when(k + 2 < KP)(lambda: xchunk(k + 2).start())
            if NP:
                pl.when(k + 2 == KP)(lambda: xpart().start())
            pl.when(k % 2 == 0)(lambda: block(k, ya, yb))
            pl.when(k % 2 == 1)(lambda: block(k, yb, ya))
            pl.when(k == 2)(lambda: ofirst.wait())
            pl.when(k > 2)(lambda: ochunk(k - 2).wait())
            pl.when(k == 0)(lambda: ofirst.start())
            pl.when(k > 0)(lambda: ochunk(k).start())
            return 0

        lax.fori_loop(0, NBLK, body, 0)

        acc = xf[(H - 1 + 2) % RING, :, HW:] + jnp.concatenate([wtap(xf, 12, slice(0, C))] * 2, axis=1)
        for kk in range(NK):
            acc = acc + mm(pltpu.bitcast(w2s[kk], BF16), gs[kk * 128:(kk + 1) * 128, :])
        obuf[NBLK % NOB, 0, :, HW:] = acc.astype(o_hbm.dtype)
        olast.start()
        ochunk(NBLK - 2).wait()
        ochunk(NBLK - 1).wait()
        olast.wait()

    return kernel, RING


_U = 8
_SCHED = {'c': (3.08, 7.0, 9.92, 13.33, 16.75, 20.17, 24.08, 28.0, 31.42, 34.83, 38.25, 40.67), 'upfree': 1, 'up': (3.0, 4.5, 4.5, 9.0, 10.5, 12.0), 'ld': (7.5, 5.5), 'w2dt': (4, 2, 4, 4, 4, 4), 'roff': (-1, -1), 'nrp': 4, 'mode': 0, 'early': 1, 'noxf': 1, 'wino': 1, 'half': 0, 'nodma': 0, 'side': 0, 'zdt': 2, 'ydt': 5, 'rtok': 0, 'rwin': 2, 'uwin': 0, 'both': 0, 'ldb': (8.0, 5.5), 'rgap': 0, 'casc': 0, 'w1c': ((24, 2),)}


@jax.jit
def pallas_standalone__modern_conv_block_convnext__vision_kernel(x, dw, w1, b1, w2, b2, gamma):
    U, O, FLAGS = _U, _SCHED, (('XLA_TPU_EVENLY_DISTRIBUTE_CRITICAL_NODES', True),)
    B, H, W, C = x.shape
    E = w1.shape[1]
    xt = jnp.transpose(x[0], (0, 2, 1))
    args = (dw, w1, b1.reshape(1, E), w2.T, b2.reshape(1, C), gamma.reshape(1, C))
    kern, RING = _make(H, C, W, E, U, dict(O))
    vm = pl.BlockSpec(memory_space=pltpu.VMEM)
    out = pl.pallas_call(
        kern,
        in_specs=[pl.BlockSpec(memory_space=pl.ANY)] + [vm for a in args],
        out_specs=pl.BlockSpec(memory_space=pl.ANY),
        out_shape=jax.ShapeDtypeStruct((H, C, W), x.dtype),
        scratch_shapes=[
            pltpu.VMEM((9, U, C, W), BF16),
            pltpu.SemaphoreType.DMA((4,)),
            pltpu.SemaphoreType.DMA((4,)),
            pltpu.VMEM((2, E // 2, 128), U32),
            pltpu.VMEM((E // 128 + 1, C // 2, 128), U32),
            pltpu.VMEM((RING + 4, C, W), F32),
            pltpu.VMEM((U + 1, C, W), F32),
            pltpu.VMEM((U + 1, C, W), F32),
            pltpu.VMEM((5, C, W // 2), F32),
            pltpu.VMEM((E + 8, W // 2), F32),
            pltpu.SMEM((3,), jnp.int32),
        ],
        compiler_params=pltpu.CompilerParams(vmem_limit_bytes=96 * 1024 * 1024, flags=dict(FLAGS), disable_bounds_checks=bool(dict(O).get('nobc', 1))),
    )(xt, *args)
    return jnp.transpose(out, (0, 2, 1))[None]
```

```python
import functools
import jax
import jax.numpy as jnp
from jax import lax
import jax.experimental.pallas as pl
import jax.experimental.pallas.tpu as pltpu
import numpy as np

_K0 = float(np.sqrt(2.0 / np.pi))
_K1 = _K0 * 0.044715
_A = _K1 ** (1.0 / 3.0)
_C0 = _K0 / _A
_EPS = 1e-5
F32 = jnp.float32
BF16 = jnp.bfloat16
U32 = jnp.uint32


def _make(H, C, W, E, U, o):
    NBLK = H // U
    NT = W // 128
    NCG = C // 8
    NK = E // 128
    NUP = 6
    WINO = 0
    NWT = 12 if WINO else 9
    XL = o.get('xl', 1) + WINO
    LA = U + 2 + XL
    RING = 4 * U
    NXB = 4
    NOB = 4
    HW = W // 2
    NRP = o.get('nrp', 4)
    MODE = o.get('mode', 3)
    assert NBLK % 2 == 0

    def kernel(x_hbm, dw_hbm, w1_hbm, b1_hbm, w2t_hbm, b2_hbm, g_hbm, o_hbm,
               io, xsem, osem, w1s, w2s, xf, ya, yb, accx, gs, zs,
               w1_ref, w2t_ref, dw_ref, b1_ref, b2_ref, g_ref, psem, pad):

        xbuf = io.at[pl.ds(0, 5)]
        obuf = io.at[pl.ds(5, 4)]

        def xchunk(k):
            s_ = k % NXB
            return pltpu.make_async_copy(x_hbm.at[pl.ds(k * U + LA, U)], xbuf.at[s_], xsem.at[s_])

        KP = (H - LA) // U
        NP = H - LA - KP * U

        def xpart():
            return pltpu.make_async_copy(x_hbm.at[pl.ds(H - NP, NP)], xbuf.at[KP % NXB, pl.ds(0, NP)], xsem.at[KP % NXB])

        def ochunk(k):
            s_ = k % NOB
            return pltpu.make_async_copy(obuf.at[s_], o_hbm.at[pl.ds(k * U - 1, U)], osem.at[s_])

        ofirst = pltpu.make_async_copy(obuf.at[0, pl.ds(1, U - 1)], o_hbm.at[pl.ds(0, U - 1)], osem.at[0])
        olast = pltpu.make_async_copy(obuf.at[NBLK % NOB, pl.ds(0, 1)], o_hbm.at[pl.ds(H - 1, 1)], osem.at[NBLK % NOB])

        def tiles(v):
            return [v[:, t * 128:(t + 1) * 128] for t in range(NT)]

        def wtap(ref, k, cs):
            return ref[RING + k // 4, cs, (k % 4) * 128:(k % 4) * 128 + 128]

        def conv_piece(cg, x0, x1, x2, wref, want_z=False, wino=False):
            lane = lax.broadcasted_iota(jnp.int32, (8, 128), 1)
            cs = slice(cg * 8, cg * 8 + 8)
            wv = [wtap(wref, k, cs) for k in range(9)]
            x0, x1, x2 = tiles(x0), tiles(x1), tiles(x2)
            z = [[x0[t] * wv[b] + x1[t] * wv[3 + b] + x2[t] * wv[6 + b] for t in range(NT)] for b in range(3)]
            if o.get('casc', 0):
                L1 = [pltpu.roll(v, 127, 1) for v in z[1]]
                L2 = [pltpu.roll(v, 127, 1) for v in z[2]]
                bb = [z[0][t] + jnp.where(lane == 127, L1[t + 1] if t < NT - 1 else 0.0, L1[t]) for t in range(NT)]
                Rb = [pltpu.roll(v, 1, 1) for v in bb]
                out = [jnp.where(lane == 0, Rb[t - 1] if t > 0 else z[1][0], Rb[t])
                       + jnp.where(lane == 127, L2[t + 1] if t < NT - 1 else 0.0, L2[t]) for t in range(NT)]
            else:
                Rr = [pltpu.roll(v, 1, 1) for v in z[0]]
                Ll = [pltpu.roll(v, 127, 1) for v in z[2]]
                out = []
                for t in range(NT):
                    lt = jnp.where(lane == 0, Rr[t - 1] if t > 0 else 0.0, Rr[t])
                    rt = jnp.where(lane == 127, Ll[t + 1] if t < NT - 1 else 0.0, Ll[t])
                    out.append(z[1][t] + lt + rt)
            return (out, z) if want_z else out

        def direct_front(cg, d, wref):
            cs = slice(cg * 8, cg * 8 + 8)
            wv = [wtap(wref, k, cs) for k in range(9)]
            n = d[0].shape[1] // 128
            d = [[v[:, t * 128:(t + 1) * 128] for t in range(n)] for v in d]
            return [[d[0][t] * wv[b] + d[1][t] * wv[3 + b] + d[2][t] * wv[6 + b] for t in range(n)] for b in range(3)]

        def wino_front(cg, d, wref):
            cs = slice(cg * 8, cg * 8 + 8)
            wv = [wtap(wref, k, cs) for k in range(12)]
            n = d[0].shape[1] // 128
            d = [[v[:, t * 128:(t + 1) * 128] for t in range(n)] for v in d]
            T = [(d[0][t] - d[2][t], d[1][t] + d[2][t], d[2][t] - d[1][t], d[1][t] - d[3][t]) for t in range(n)]
            z = [[[], [], []], [[], [], []]]
            for b in range(3):
                for t in range(n):
                    m0, m1, m2, m3 = (T[t][k] * wv[k * 3 + b] for k in range(4))
                    z[0][b].append(m0 + m1 + m2)
                    z[1][b].append(m1 - m2 - m3)
            return z

        def shift_sum(z1, Rr, Ll, t):
            lane = lax.broadcasted_iota(jnp.int32, (8, 128), 1)
            lt = jnp.where(lane == 0, Rr[t - 1] if t > 0 else 0.0, Rr[t])
            rt = jnp.where(lane == 127, Ll[t + 1] if t < NT - 1 else 0.0, Ll[t])
            return z1[t] + lt + rt

        def fold4(v):
            s = lax.broadcasted_iota(jnp.int32, (8, 128), 0)
            m4 = s < 4
            m2 = (s & 2) == 0
            a = jnp.where(m4, v[0], v[1]) + pltpu.roll(jnp.where(m4, v[1], v[0]), 4, 0)
            b = jnp.where(m4, v[2], v[3]) + pltpu.roll(jnp.where(m4, v[3], v[2]), 4, 0)
            w = jnp.where(m2, a + pltpu.roll(a, 6, 0), b + pltpu.roll(b, 2, 0))
            return w + pltpu.roll(w, 7, 0)

        def rstd4(s1, s2):
            m = fold4(s1) * (1.0 / C)
            q = fold4(s2) * (1.0 / C)
            return lax.rsqrt(jnp.maximum(q - m * m, 0.0) + _EPS)

        def pick(rs, t):
            sl = (0, 4, 2, 6)[t]
            return rs[sl:sl + 1, :]

        def aug(hn):
            n = hn.shape[1]
            r8 = lax.broadcasted_iota(jnp.int32, (8, n), 0)
            ones = jnp.where(r8 < 2, 1.0, 0.0).astype(F32)
            return jnp.concatenate([hn, ones, jnp.zeros((128 - C - 8, n), F32)], axis=0)

        zs[0] = 0
        zs[1] = 0
        zs[2] = 0
        LX = LA - U
        head = pltpu.make_async_copy(x_hbm.at[pl.ds(0, U)], xbuf.at[NXB - 1], xsem.at[NXB - 1])
        head2 = pltpu.make_async_copy(x_hbm.at[pl.ds(U, LX)], obuf.at[NOB - 1, pl.ds(0, LX)], osem.at[NOB - 1])
        params = [pltpu.make_async_copy(a, b, psem.at[n]) for n, (a, b) in enumerate(
            [(dw_hbm, dw_ref), (w1_hbm, w1_ref), (b1_hbm, b1_ref), (w2t_hbm, w2t_ref), (b2_hbm, b2_ref), (g_hbm, g_ref)])]
        for c in params:
            c.start()
        head.start()
        head2.start()
        gs[...] = jnp.zeros(gs.shape, F32)
        xf[0] = jnp.zeros((C, W), F32)
        xf[1] = jnp.zeros((C, W), F32)
        for c in params:
            c.wait()
        pad[...] = dw_ref[...]
        rows = [(pad if o.get('pad', 1) and a == 0 else dw_ref)[a, b:b + 1, :].astype(F32) for a in range(3) for b in range(3)]
        plain = list(rows)
        if WINO:
            g0, g1, g2 = rows[0:3], rows[3:6], rows[6:9]
            rows = g0 + [(a + b + c) * 0.5 for a, b, c in zip(g0, g1, g2)] + [(a - b + c) * 0.5 for a, b, c in zip(g0, g1, g2)] + g2
        rows.append(b2_ref[...].astype(F32))
        rows.append(g_ref[...].astype(F32))
        p = jnp.concatenate(rows + [jnp.zeros((128 - len(rows), C), F32)], axis=0)
        p = jnp.concatenate([p, jnp.zeros((128, 128 - C), F32)], axis=1)
        pt = p.T
        for k in range(NWT):
            xf[RING + k // 4, :, (k % 4) * 128:(k % 4) * 128 + 128] = jnp.broadcast_to(pt[:C, k:k + 1], (C, 128))
        gcol = pt[:C, NWT + 1:NWT + 2]
        xf[RING + 3, :, 0:128] = jnp.broadcast_to(pt[:C, NWT:NWT + 1] * gcol, (C, 128))
        w2f = (w2t_ref[...].astype(F32) * (gcol * (0.5 / _A))).astype(BF16)
        for k in range(NK):
            w2s[k] = pltpu.bitcast(w2f[:, k * 128:(k + 1) * 128], U32)
        w1 = w1_ref[...].astype(F32)
        w1c = (w1 - jnp.mean(w1, axis=0, keepdims=True)) * _A
        b1 = b1_ref[...].astype(F32).reshape(1, E) * _A
        b1h = b1.astype(BF16).astype(F32)
        b1l = b1 - b1h
        r8 = lax.broadcasted_iota(jnp.int32, (8, E), 0)
        tail = jnp.where(r8 == 0, b1h, jnp.where(r8 == 1, b1l, 0.0))
        waug = jnp.concatenate([w1c, tail, jnp.zeros((128 - C - 8, E), F32)], axis=0)
        wt = waug.T
        wt = jnp.concatenate([wt[kk * 128 + j * 8:kk * 128 + j * 8 + 8] for kk in range(NK) for j in reversed(range(16))], axis=0)
        w1s[0] = pltpu.bitcast(wt.astype(BF16), U32)
        head.wait()
        head2.wait()
        xchunk(0).start()
        xchunk(1).start()
        PR = o.get('pr', U)
        s1 = {}
        s2 = {}
        for r0_ in range(0, U, PR):
            for cg in range(NCG):
                cs = slice(cg * 8, cg * 8 + 8)

                def row(r):
                    if r < 0:
                        return jnp.zeros((8, W), F32)
                    v = (xbuf[NXB - 1, r, cs, :] if r < U else obuf[NOB - 1, r - U, cs, :]).astype(F32)
                    xf[r + 2, cs, :] = v
                    return v
                xs = {r: row(r) for r in range(r0_ - 1, r0_ + PR + 1)}
                if r0_ + PR == U:
                    for r in range(U + 1, LA):
                        row(r)
                for r in range(r0_, r0_ + PR):
                    y = conv_piece(cg, xs[r - 1], xs[r], xs[r + 1], xf)
                    ya[r, cs, :] = jnp.concatenate(y, axis=1)
                    s1[r] = y if cg == 0 else [a + b for a, b in zip(s1[r], y)]
                    s2[r] = [b * b if cg == 0 else a + b * b for a, b in zip(s2.get(r, y), y)]
            for r in range(r0_, r0_ + PR):
                ya[U, (r % 12) * 8:(r % 12) * 8 + 8, 128 + 128 * (r // 12):256 + 128 * (r // 12)] = rstd4(s1[r], s2[r])

        mm = lambda a, b: lax.dot_general(a, b, (((1,), (0,)), ((), ())), preferred_element_type=F32)

        def gelu(zz):
            tt = zz * (zz * zz + _C0)
            return zz * jnp.tanh(tt) + zz

        ZP = o.get('zp', 0)

        def parked(v, kk):
            if kk < NK - 1 or ZP == 0:
                return v
            return jnp.concatenate([gelu(v[:ZP * 8]), v[ZP * 8:]], axis=0)

        def rev(g, kk):
            return jnp.concatenate([g[kk * 128 + j * 8:kk * 128 + j * 8 + 8] for j in reversed(range(16))], axis=0)

        def block(k, ycur, ynxt):
            r0 = k * U
            z0 = zs[0]
            z1 = zs[1]
            z2 = zs[2]
            src = xbuf.at[k % NXB]
            ocur = obuf.at[k % NOB]
            onxt = obuf.at[(k + 1) % NOB]
            wd = xf.at[pl.ds(z0, RING + 4)]
            ybd = ycur.at[pl.ds(z0, U + 1)]
            rbase = (k % 4) * U + 1

            def ring(r):
                return (rbase + r + 1) & (RING - 1)

            ev = []
            st = dict(n=0, s1=None, s2=None, z=None, up=LA, nup=0, out=[])
            evr = []
            ev2 = []
            vals = {}

            def token(T, wide=False, side=False):
                c = [e for e in ev if e[0] <= T + 1e-6]
                if o.get('notok', 0):
                    return None
                if side:
                    late = max([e[0] for e in c], default=-99)
                    c += [e for e in ev2 if late + 1.0 < e[0] <= T + 1e-6]
                if not c:
                    return None
                _, a, j = max(c, key=lambda e: e[0])
                return a[j * 8:j * 8 + 8, 0:256].astype(BF16) if wide else a[j * 8:j * 8 + 8, 0:128]

            def xtok(v, T=None):
                c = [e for e in evr if T is not None and T - o.get('rwin', 2) <= e[0] <= T]
                if c:
                    for e in c:
                        xf[RING + 3 + z2, 0:8, 384:512] = e[1]
                        evr.remove(e)
                    if not o.get('both', 0):
                        return
                xf[RING + 3 + z2, 0:8, 384:512] = v

            def conv_next(v_, T=None):
                v, n = divmod(st['n'], NCG)
                if st['n'] >= U * NCG * (1 + o.get('half', 0)):
                    return
                if v_ is not None:
                    xtok(v_, T)
                if o.get('half', 0):
                    v, n, part = st['n'] // 24, (st['n'] % 24) // 2, st['n'] % 2
                    assert v + U + 1 < st['up'], (v, st['up'])
                    cs = slice(n * 8, n * 8 + 8)
                    ts = slice(part * HW, part * HW + HW)
                    z = direct_front(n, [xf[ring(v + U - 1 + q), cs, ts] for q in range(3)], wd)
                    st['z'] = [None, [None, None, z[1][1]]]
                    zz_ = st['zk'] if part else [[], [], []]
                    zz_[0] += [pltpu.roll(a, 1, 1) for a in z[0]]
                    zz_[1] += z[1]
                    zz_[2] += [pltpu.roll(a, 127, 1) for a in z[2]]
                    st['zk'] = zz_
                    if part == 0:
                        st['y0'] = shift_sum(zz_[1], zz_[0], zz_[2], 0)
                    else:
                        finish(v, n, [st['y0']] + [shift_sum(zz_[1], zz_[0], zz_[2], t) for t in range(1, NT)], 0)
                elif WINO:
                    v, n, part = 2 * (st['n'] // 24), (st['n'] % 24) // 2, st['n'] % 2
                    assert v + U + 2 < st['up'], (v, st['up'])
                    cs = slice(n * 8, n * 8 + 8)
                    ts = slice(part * HW, part * HW + HW)
                    z = wino_front(n, [xf[ring(v + U - 1 + q), cs, ts] for q in range(4)], wd)
                    st['z'] = [None, [None, None, z[1][1][1]]]
                    zz_ = st['zk'] if part else [[[], [], []], [[], [], []]]
                    for q in range(2):
                        zz_[q][0] += [pltpu.roll(a, 1, 1) for a in z[q][0]]
                        zz_[q][1] += z[q][1]
                        zz_[q][2] += [pltpu.roll(a, 127, 1) for a in z[q][2]]
                    st['zk'] = zz_
                    if part == 0:
                        st['y0'] = [shift_sum(zz_[q][1], zz_[q][0], zz_[q][2], 0) for q in range(2)]
                    else:
                        for q in range(2):
                            y = [st['y0'][q]] + [shift_sum(zz_[q][1], zz_[q][0], zz_[q][2], t) for t in range(1, NT)]
                            finish(v + q, n, y, q)
                else:
                    assert v + U + 1 < st['up'], (v, st['up'])
                    cs = slice(n * 8, n * 8 + 8)
                    y, st['z'] = conv_piece(n, xf[ring(v + U - 1), cs, :], xf[ring(v + U), cs, :], xf[ring(v + U + 1), cs, :], wd, True)
                    finish(v, n, y, 0)
                    if T is not None:
                        ev2.append((T + o.get('zdt', 2), st['z'][1][3], 0))
                        ev2.append((T + o.get('ydt', 5), y[3], 0))
                st['n'] += 1

            def finish(v, n, y, q):
                ynxt[v, n * 8:n * 8 + 8, :] = jnp.concatenate(y, axis=1)
                if n == 0:
                    st['s1', q], st['s2', q] = y, [b * b for b in y]
                else:
                    if not o.get('hack4', 0): st['s1', q] = [a + b for a, b in zip(st['s1', q], y)]
                    if not o.get('hack3', 0): st['s2', q] = [a + b * b for a, b in zip(st['s2', q], y)]
                if n == NCG - 1:
                    ynxt[U, (v % 12) * 8:(v % 12) * 8 + 8, 128 + 128 * (v // 12):256 + 128 * (v // 12)] = rstd4(st['s1', q], st['s2', q])

            def run(T, kind, u, h, n):
                if kind == 'c':
                    v = token(T)
                    conv_next(v if v is not None or st['z'] is None or o.get('notok', 0) else st['z'][1][2], T)
                elif kind == 'z':
                    conv_next(None if st['z'] is None else st['z'][1][2])
                elif kind == 'up':
                    c = [e for e in st['out'] if T - o.get('uwin', 0) <= e[0] <= T]
                    v = c[-1][1] if c else None if o.get('upfree', 0) and T > 8 else token(T, True)
                    if v is not None:
                        xbuf[NXB + z1, 0, 0:8, 0:256] = v
                    cs = slice(n * (C // NUP), (n + 1) * (C // NUP))
                    xf[ring(st['up']), cs, :] = src[u, cs, :].astype(F32)
                    st['nup'] += 1
                    if n == NUP - 1:
                        st['up'] += 1
                elif kind == 'ld':
                    v = token(T)
                    if v is not None:
                        ycur[U + z1, 0:8, 0:128] = v
                    if ('rs', u) not in vals:
                        vals['rs', u] = ybd[U, (u % 12) * 8:(u % 12) * 8 + 8, 128 + 128 * (u // 12):256 + 128 * (u // 12)]
                    t = 2 * h + n
                    vals['h', u, t] = ybd[u, :, t * 128:(t + 1) * 128] * pick(vals['rs', u], t)
                elif kind == 'w1':
                    v = token(T, side=o.get('side', 0))
                    if v is not None:
                        w1s[1 + z1, 0:8, :] = pltpu.bitcast(v, U32)
                    a0, a1 = n
                    vals.setdefault(('w1', u, h), []).append(w1s[z0, a0 * 8:a1 * 8, :])
                elif kind == 'w2':
                    v = token(T)
                    if v is not None:
                        w2s[NK + z1, 0:8, :] = pltpu.bitcast(v, U32)
                    vals['w2', u, h, n] = w2s[n + z0]
                elif kind == 'gl':
                    v = token(T)
                    if v is not None:
                        gs[E + z1 * 8:E + z1 * 8 + 8, 0:128] = v
                    vals['g', u, h, n] = parked(gs[pl.ds(pl.multiple_of(z0 * 8 + n * 128, 8), 128), :], n)
                elif kind == 'gp':
                    m = (n // 16) * 16 + 15 - n % 16
                    gs[m * 8:m * 8 + 8, :] = vals['graw' if n < 48 - o.get('zp', 0) else 'zraw'][n * 8:n * 8 + 8, :]
                elif kind == 'pk':
                    kk, q = n
                    nr = C // NRP
                    rs8 = slice(q * nr, q * nr + nr)
                    P = vals['P', u, h]
                    if MODE == 3:
                        accx[2 * h + kk + z1, rs8, :] = P[kk][rs8]
                    elif MODE == 5:
                        if kk == 0:
                            accx[2 * h + z1, rs8, :] = P[0][rs8]
                    elif MODE == 0:
                        pass
                    elif kk == 1:
                        accx[2 * h + z1, rs8, :] = P[0][rs8] + P[1][rs8]
                elif kind == 'r':
                    v = token(T)
                    if v is not None:
                        if not o.get('noxf', 0):
                            xtok(v)
                        if MODE != 0:
                            accx[4 + z1, 0:8, 0:128] = v
                    nr = C // NRP
                    rs8 = slice(n * nr, n * nr + nr)
                    hs = slice(h * HW, h * HW + HW)
                    gbv = wtap(wd, 12, rs8)
                    res = xf[ring(u), rs8, hs] + jnp.concatenate([gbv, gbv], axis=1)
                    P = vals['P', u, h]
                    if MODE == 0:
                        a = (P[0][rs8] + P[1][rs8]) + res
                        if o.get('hack2', 0):
                            a = (P[0][rs8] + P[1][rs8])
                    elif MODE == 5:
                        a = (accx[2 * h + z0, rs8, :] + res) + P[1][rs8]
                    else:
                        a = accx[2 * h + z0, rs8, :] + res
                    if MODE == 3:
                        a = a + accx[2 * h + 1 + z0, rs8, :]
                    outf = a + vals['P', u, h][2][rs8]
                    out = outf.astype(o_hbm.dtype)
                    st['out'].append((T, out[nr - 8:nr, :]))
                    if o.get('rtok', 0):
                        for t_ in range(o['rtok']):
                            evr.append((T + 0.02, outf[nr - 8 * (1 + t_ // 2):, 128 * (1 - t_ % 2):][0:8, 0:128]))
                    if u + 1 < U:
                        ocur[u + 1, rs8, hs] = out
                    else:
                        onxt[0, rs8, hs] = out

            S0 = ((0.0, 0.0), (18.0, 0.0))
            items = []
            w1items = {}
            add = lambda T, kind, u, h, n: items.append((T, len(items), kind, u, h, n))
            for e in range(o.get('early', 0)):
                add(o['et'][e] if 'et' in o else -20 + e, 'z', 0, 0, 0)
            m2start = lambda u, h: 42 * u + (24 if h == 0 else 42)
            for u in range(-1, U):
                if u >= 0:
                    for j, tau in enumerate(o.get('cf' if u == 0 else 'cl' if u == U - 1 else 'c', o['c'])):
                        if (u, j) not in o.get('skip', ()):
                            add(42 * u + tau, 'c', u, 0, 0)
                    for n in range(NUP):
                        add(42 * u + o.get('upf' if u == 0 else 'up', o['up'])[n], 'up', u, 0, n)
                for h in range(2):
                    if u >= 0:
                        m1 = 42 * u + S0[h][0]
                        for n in range(2):
                            add(m1 - (o['ld'] if h == 0 else o.get('ldb', o['ld']))[n], 'ld', u, h, n)
                        a0 = 0
                        for nst, dt in (o['w1c'] if h == 0 else o.get('w1b', o['w1c'])):
                            w1items.setdefault((u, h), []).append((m1 + a0 - dt, 'w1', u, h, (a0, a0 + nst)))
                            a0 += nst
                    if (u == U - 1 and h == 1):
                        for j in range(48):
                            add(42 * u + 27 + j / 2, 'gp', u, h, j)
                        continue
                    if (u == -1 and h == 0):
                        continue
                    m2 = m2start(u, h)
                    w = 6.0 / NRP
                    for kk in range(NK):
                        add(m2 + 6 * kk - (o['w2dt'][3 * h + kk] if isinstance(o['w2dt'], tuple) else o['w2dt']), 'w2', u, h, kk)
                        if u == -1:
                            add(m2 + 6 * kk - o.get('gldt', (6, 6, 6))[kk], 'gl', u, h, kk)
                        if kk < 2:
                            for q in range(NRP):
                                add(m2 + 8 + 6 * kk + (q + 1) * w - 0.5, 'pk', u, h, (kk, q))
                    for q in range(NRP):
                        add(m2 + 20 + q * w + (o['roff'][h] if isinstance(o['roff'], tuple) else o['roff']) + o.get('rgap', 0) * q, 'r', u, h, q)
            items.sort()
            ptr = [0]

            def flush(pred):
                last = max([i_ for i_, it in enumerate(items) if pred(it)], default=-1)
                while ptr[0] <= last:
                    T, _, kind, u, h, n = items[ptr[0]]
                    run(T, kind, u, h, n)
                    ptr[0] += 1

            def mat1(u, h):
                flush(lambda it: (it[2] == 'ld' and it[3] == u and it[4] == h) or (o.get('side', 0) and it[2] == 'c' and it[0] < 42 * u + S0[h][0] + (8 if h == 0 else 5)))
                for it in w1items[u, h]:
                    run(*it)
                lhs = jnp.concatenate(vals['w1', u, h], axis=0)
                if o.get('hack1', 0):
                    lhs = jnp.concatenate([lhs[0:48]] * 4, axis=0)
                rhs = jnp.concatenate([vals['h', u, 2 * h], vals['h', u, 2 * h + 1]], axis=1)
                zz = mm(pltpu.bitcast(lhs, BF16), aug(rhs))
                g = gelu(zz)
                vals['graw'] = g
                vals['zraw'] = zz
                for kk in range(NK):
                    vals['g', u, h, kk] = rev(g, kk)
                ev.extend((42 * u + S0[h][0] + 9 + j / 2, g, j) for j in range(48))

            def mat2(u, h):
                flush(lambda it: it[2] in ('w2', 'gl') and it[3] == u and it[4] == h)
                P = [mm(pltpu.bitcast(vals['w2', u, h, kk], BF16), vals['g', u, h, kk]) for kk in range(NK)]
                vals['P', u, h] = P
                ev.extend((m2start(u, h) + 8 + 6 * kk + j / 2 + 0.01, P[kk], j) for kk in range(NK) for j in range(12))

            for u in range(U):
                mat1(u, 0)
                mat2(u - 1, 1)
                mat1(u, 1)
                mat2(u, 0)
            flush(lambda it: True)
            assert st['n'] == U * NCG * (1 + o.get('half', 0)) and st['up'] == LA + U, st

        def body(k, _):
            pl.when(k < KP)(lambda: xchunk(k).wait())

            @pl.when(k == KP)
            def _():
                if NP:
                    xpart().wait()
                xbuf[KP % NXB, NP] = jnp.zeros((C, W), BF16)

            pl.when(k + 2 < KP)(lambda: xchunk(k + 2).start())
            if NP:
                pl.when(k + 2 == KP)(lambda: xpart().start())
            pl.when(k % 2 == 0)(lambda: block(k, ya, yb))
            pl.when(k % 2 == 1)(lambda: block(k, yb, ya))
            pl.when(k == 2)(lambda: ofirst.wait())
            pl.when(k > 2)(lambda: ochunk(k - 2).wait())
            pl.when(k == 0)(lambda: ofirst.start())
            pl.when(k > 0)(lambda: ochunk(k).start())
            return 0

        lax.fori_loop(0, NBLK, body, 0)

        acc = xf[(H - 1 + 2) % RING, :, HW:] + jnp.concatenate([wtap(xf, 12, slice(0, C))] * 2, axis=1)
        for kk in range(NK):
            acc = acc + mm(pltpu.bitcast(w2s[kk], BF16), parked(gs[kk * 128:(kk + 1) * 128, :], kk))
        obuf[NBLK % NOB, 0, :, HW:] = acc.astype(o_hbm.dtype)
        olast.start()
        ochunk(NBLK - 2).wait()
        ochunk(NBLK - 1).wait()
        olast.wait()

    return kernel, RING


_U = 8
_SCHED = {'c': (3.08, 7.0, 9.92, 13.33, 16.75, 20.17, 24.08, 28.0, 31.42, 34.83, 38.25, 40.67), 'upfree': 1, 'up': (3.0, 4.5, 4.5, 9.0, 10.5, 12.0), 'ld': (7.5, 5.5), 'w2dt': (6, 2, 4, 4, 4, 4), 'roff': (-1, -1), 'nrp': 4, 'mode': 0, 'early': 1, 'noxf': 1, 'wino': 1, 'half': 0, 'nodma': 0, 'side': 0, 'zdt': 2, 'ydt': 5, 'rtok': 0, 'rwin': 2, 'uwin': 0, 'both': 0, 'ldb': (8.0, 5.5), 'rgap': -0.25, 'casc': 0, 'zp': 8, 'gldt': (6, 6, 6), 'cf': (3.08, 7.0, 9.92, 13.83, 15.75, 20.17, 23.08, 27.0, 31.42, 34.83, 38.25, 40.67), 'cl': (3.08, 7.0, 9.92, 13.33, 15.75, 20.17, 24.08, 28.0, 32.92, 34.83, 38.25, 39.67), 'upf': (3.0, 4.5, 4.5, 9.0, 10.5, 12.0), 'w1c': ((24, 2),)}


@jax.jit
def pallas_standalone__modern_conv_block_convnext__vision_kernel(x, dw, w1, b1, w2, b2, gamma):
    U, O, FLAGS = _U, _SCHED, (('XLA_TPU_EVENLY_DISTRIBUTE_CRITICAL_NODES', True),)
    B, H, W, C = x.shape
    E = w1.shape[1]
    xt = jnp.transpose(x[0], (0, 2, 1))
    args = (dw, w1, b1, w2.T, b2.reshape(1, C), gamma.reshape(1, C))
    kern, RING = _make(H, C, W, E, U, dict(O))
    vm = pl.BlockSpec(memory_space=pltpu.VMEM)
    out = pl.pallas_call(
        kern,
        in_specs=[pl.BlockSpec(memory_space=pl.ANY)] + [pl.BlockSpec(memory_space=pl.ANY) for a in args],
        out_specs=pl.BlockSpec(memory_space=pl.ANY),
        out_shape=jax.ShapeDtypeStruct((H, C, W), x.dtype),
        scratch_shapes=[
            pltpu.VMEM((9, U, C, W), BF16),
            pltpu.SemaphoreType.DMA((4,)),
            pltpu.SemaphoreType.DMA((4,)),
            pltpu.VMEM((2, E // 2, 128), U32),
            pltpu.VMEM((E // 128 + 1, C // 2, 128), U32),
            pltpu.VMEM((RING + 4, C, W), F32),
            pltpu.VMEM((U + 1, C, W), F32),
            pltpu.VMEM((U + 1, C, W), F32),
            pltpu.VMEM((5, C, W // 2), F32),
            pltpu.VMEM((E + 8, W // 2), F32),
            pltpu.SMEM((3,), jnp.int32),
        ] + [pltpu.VMEM(args[n].shape, args[n].dtype) for n in (1, 3, 0, 2, 4, 5)] + [pltpu.SemaphoreType.DMA((len(args),)), pltpu.VMEM(args[0].shape, args[0].dtype)],
        compiler_params=pltpu.CompilerParams(vmem_limit_bytes=96 * 1024 * 1024, flags=dict(FLAGS), disable_bounds_checks=bool(dict(O).get('nobc', 1))),
    )(xt, *args)
    return jnp.transpose(out, (0, 2, 1))[None]
```

```python
import functools
import jax
import jax.numpy as jnp
from jax import lax
import jax.experimental.pallas as pl
import jax.experimental.pallas.tpu as pltpu
import numpy as np

_K0 = float(np.sqrt(2.0 / np.pi))
_K1 = _K0 * 0.044715
_A = _K1 ** (1.0 / 3.0)
_C0 = _K0 / _A
_EPS = 1e-5
F32 = jnp.float32
BF16 = jnp.bfloat16
U32 = jnp.uint32


def _make(H, C, W, E, U, o):
    NBLK = H // U
    NT = W // 128
    NCG = C // 8
    NK = E // 128
    NUP = 6
    WINO = o.get('wino_', 0)
    NWT = 12 if WINO else 9
    XL = o.get('xl', 1) + WINO
    LA = U + 2 + XL
    RING = 4 * U
    NXB = 4
    NOB = 4
    HW = W // 2
    NRP = o.get('nrp', 4)
    MODE = o.get('mode', 3)
    assert NBLK % 2 == 0

    def low2(k):
        return k % 4 if isinstance(k, int) else k & 3

    def kernel(x_hbm, dw_hbm, w1_hbm, b1_hbm, w2t_hbm, b2_hbm, g_hbm, o_hbm,
               io, xsem, osem, w1s, w2s, xf, ya, yb, accx, gs, zs,
               w1_ref, w2t_ref, dw_ref, b1_ref, b2_ref, g_ref, psem, pad):

        xbuf = io.at[pl.ds(0, 5)]
        obuf = io.at[pl.ds(5, 4)]

        def xchunk(k):
            s_ = low2(k)
            return pltpu.make_async_copy(x_hbm.at[pl.ds(k * U + LA, U)], xbuf.at[s_], xsem.at[s_])

        KP = (H - LA) // U
        NP = H - LA - KP * U

        def xpart():
            return pltpu.make_async_copy(x_hbm.at[pl.ds(H - NP, NP)], xbuf.at[KP % NXB, pl.ds(0, NP)], xsem.at[KP % NXB])

        def ochunk(k):
            s_ = low2(k)
            return pltpu.make_async_copy(obuf.at[s_], o_hbm.at[pl.ds(k * U - 1, U)], osem.at[s_])

        ofirst = pltpu.make_async_copy(obuf.at[0, pl.ds(1, U - 1)], o_hbm.at[pl.ds(0, U - 1)], osem.at[0])
        olast = pltpu.make_async_copy(obuf.at[NBLK % NOB, pl.ds(0, 1)], o_hbm.at[pl.ds(H - 1, 1)], osem.at[NBLK % NOB])

        def tiles(v):
            return [v[:, t * 128:(t + 1) * 128] for t in range(NT)]

        def wtap(ref, k, cs):
            return ref[RING + k // 4, cs, (k % 4) * 128:(k % 4) * 128 + 128]

        def conv_piece(cg, x0, x1, x2, wref, want_z=False, wino=False):
            lane = lax.broadcasted_iota(jnp.int32, (8, 128), 1)
            cs = slice(cg * 8, cg * 8 + 8)
            wv = [wtap(wref, k, cs) for k in range(9)]
            x0, x1, x2 = tiles(x0), tiles(x1), tiles(x2)
            z = [[x0[t] * wv[b] + x1[t] * wv[3 + b] + x2[t] * wv[6 + b] for t in range(NT)] for b in range(3)]
            if o.get('casc', 0):
                L1 = [pltpu.roll(v, 127, 1) for v in z[1]]
                L2 = [pltpu.roll(v, 127, 1) for v in z[2]]
                bb = [z[0][t] + jnp.where(lane == 127, L1[t + 1] if t < NT - 1 else 0.0, L1[t]) for t in range(NT)]
                Rb = [pltpu.roll(v, 1, 1) for v in bb]
                out = [jnp.where(lane == 0, Rb[t - 1] if t > 0 else z[1][0], Rb[t])
                       + jnp.where(lane == 127, L2[t + 1] if t < NT - 1 else 0.0, L2[t]) for t in range(NT)]
            else:
                Rr = [pltpu.roll(v, 1, 1) for v in z[0]]
                Ll = [pltpu.roll(v, 127, 1) for v in z[2]]
                out = []
                for t in range(NT):
                    lt = jnp.where(lane == 0, Rr[t - 1] if t > 0 else 0.0, Rr[t])
                    rt = jnp.where(lane == 127, Ll[t + 1] if t < NT - 1 else 0.0, Ll[t])
                    out.append(z[1][t] + lt + rt)
            return (out, z) if want_z else out

        def direct_front(cg, d, wref):
            cs = slice(cg * 8, cg * 8 + 8)
            wv = [wtap(wref, k, cs) for k in range(9)]
            n = d[0].shape[1] // 128
            d = [[v[:, t * 128:(t + 1) * 128] for t in range(n)] for v in d]
            return [[d[0][t] * wv[b] + d[1][t] * wv[3 + b] + d[2][t] * wv[6 + b] for t in range(n)] for b in range(3)]

        def wino_front(cg, d, wref):
            cs = slice(cg * 8, cg * 8 + 8)
            wv = [wtap(wref, k, cs) for k in range(12)]
            n = d[0].shape[1] // 128
            d = [[v[:, t * 128:(t + 1) * 128] for t in range(n)] for v in d]
            T = [(d[0][t] - d[2][t], d[1][t] + d[2][t], d[2][t] - d[1][t], d[1][t] - d[3][t]) for t in range(n)]
            z = [[[], [], []], [[], [], []]]
            for b in range(3):
                for t in range(n):
                    m0, m1, m2, m3 = (T[t][k] * wv[k * 3 + b] for k in range(4))
                    z[0][b].append(m0 + m1 + m2)
                    z[1][b].append(m1 - m2 - m3)
            return z

        def shift_sum(z1, Rr, Ll, t):
            lane = lax.broadcasted_iota(jnp.int32, (8, 128), 1)
            lt = jnp.where(lane == 0, Rr[t - 1] if t > 0 else 0.0, Rr[t])
            rt = jnp.where(lane == 127, Ll[t + 1] if t < NT - 1 else 0.0, Ll[t])
            return z1[t] + lt + rt

        def fold4(v):
            s = lax.broadcasted_iota(jnp.int32, (8, 128), 0)
            m4 = s < 4
            m2 = (s & 2) == 0
            a = jnp.where(m4, v[0], v[1]) + pltpu.roll(jnp.where(m4, v[1], v[0]), 4, 0)
            b = jnp.where(m4, v[2], v[3]) + pltpu.roll(jnp.where(m4, v[3], v[2]), 4, 0)
            w = jnp.where(m2, a + pltpu.roll(a, 6, 0), b + pltpu.roll(b, 2, 0))
            return w + pltpu.roll(w, 7, 0)

        def rstd4(s1, s2):
            m = fold4(s1) * (1.0 / C)
            q = fold4(s2) * (1.0 / C)
            return lax.rsqrt(jnp.maximum(q - m * m, 0.0) + _EPS)

        def pick(rs, t):
            sl = (0, 4, 2, 6)[t]
            return rs[sl:sl + 1, :]

        def aug(hn):
            n = hn.shape[1]
            r8 = lax.broadcasted_iota(jnp.int32, (8, n), 0)
            ones = jnp.where(r8 < 2, 1.0, 0.0).astype(F32)
            return jnp.concatenate([hn, ones, jnp.zeros((128 - C - 8, n), F32)], axis=0)

        zs[0] = 0
        zs[1] = 0
        zs[2] = 0
        LX = LA - U
        head = pltpu.make_async_copy(x_hbm.at[pl.ds(0, U)], xbuf.at[NXB - 1], xsem.at[NXB - 1])
        head2 = pltpu.make_async_copy(x_hbm.at[pl.ds(U, LX)], obuf.at[NOB - 1, pl.ds(0, LX)], osem.at[NOB - 1])
        params = [pltpu.make_async_copy(a, b, psem.at[n]) for n, (a, b) in enumerate(
            [(dw_hbm, dw_ref), (w1_hbm, w1_ref), (b1_hbm, b1_ref), (w2t_hbm, w2t_ref), (b2_hbm, b2_ref), (g_hbm, g_ref)])]
        for c in params:
            c.start()
        head.start()
        head2.start()
        gs[...] = jnp.zeros(gs.shape, F32)
        xf[0] = jnp.zeros((C, W), F32)
        xf[1] = jnp.zeros((C, W), F32)
        for c in params:
            c.wait()
        pad[...] = dw_ref[...]
        rows = [(pad if o.get('pad', 1) and a == 0 else dw_ref)[a, b:b + 1, :].astype(F32) for a in range(3) for b in range(3)]
        plain = list(rows)
        if WINO:
            g0, g1, g2 = rows[0:3], rows[3:6], rows[6:9]
            rows = g0 + [(a + b + c) * 0.5 for a, b, c in zip(g0, g1, g2)] + [(a - b + c) * 0.5 for a, b, c in zip(g0, g1, g2)] + g2
        rows.append(b2_ref[...].astype(F32))
        rows.append(g_ref[...].astype(F32))
        p = jnp.concatenate(rows + [jnp.zeros((128 - len(rows), C), F32)], axis=0)
        p = jnp.concatenate([p, jnp.zeros((128, 128 - C), F32)], axis=1)
        pt = p.T
        for k in range(NWT):
            xf[RING + k // 4, :, (k % 4) * 128:(k % 4) * 128 + 128] = jnp.broadcast_to(pt[:C, k:k + 1], (C, 128))
        gcol = pt[:C, NWT + 1:NWT + 2]
        xf[RING + 3, :, 0:128] = jnp.broadcast_to(pt[:C, NWT:NWT + 1] * gcol, (C, 128))
        w2f = (w2t_ref[...].astype(F32) * (gcol * (0.5 / _A))).astype(BF16)
        for k in range(NK):
            w2s[k] = pltpu.bitcast(w2f[:, k * 128:(k + 1) * 128], U32)
        w1 = w1_ref[...].astype(F32)
        w1c = (w1 - jnp.mean(w1, axis=0, keepdims=True)) * _A
        b1 = b1_ref[...].astype(F32).reshape(1, E) * _A
        b1h = b1.astype(BF16).astype(F32)
        b1l = b1 - b1h
        r8 = lax.broadcasted_iota(jnp.int32, (8, E), 0)
        tail = jnp.where(r8 == 0, b1h, jnp.where(r8 == 1, b1l, 0.0))
        waug = jnp.concatenate([w1c, tail, jnp.zeros((128 - C - 8, E), F32)], axis=0)
        wt = waug.T
        wt = jnp.concatenate([wt[kk * 128 + j * 8:kk * 128 + j * 8 + 8] for kk in range(NK) for j in reversed(range(16))], axis=0)
        w1s[0] = pltpu.bitcast(wt.astype(BF16), U32)
        head.wait()
        head2.wait()
        xchunk(0).start()
        xchunk(1).start()
        PR = o.get('pr', U)
        s1 = {}
        s2 = {}
        for r0_ in range(0, U, PR):
            for cg in range(NCG):
                cs = slice(cg * 8, cg * 8 + 8)

                def row(r):
                    if r < 0:
                        return jnp.zeros((8, W), F32)
                    v = (xbuf[NXB - 1, r, cs, :] if r < U else obuf[NOB - 1, r - U, cs, :]).astype(F32)
                    xf[r + 2, cs, :] = v
                    return v
                xs = {r: row(r) for r in range(r0_ - 1, r0_ + PR + 1)}
                if r0_ + PR == U:
                    for r in range(U + 1, LA):
                        row(r)
                for r in range(r0_, r0_ + PR):
                    y = conv_piece(cg, xs[r - 1], xs[r], xs[r + 1], xf)
                    ya[r, cs, :] = jnp.concatenate(y, axis=1)
                    s1[r] = y if cg == 0 else [a + b for a, b in zip(s1[r], y)]
                    s2[r] = [b * b if cg == 0 else a + b * b for a, b in zip(s2.get(r, y), y)]
            for r in range(r0_, r0_ + PR):
                ya[U, (r % 12) * 8:(r % 12) * 8 + 8, 128 + 128 * (r // 12):256 + 128 * (r // 12)] = rstd4(s1[r], s2[r])

        mm = lambda a, b: lax.dot_general(a, b, (((1,), (0,)), ((), ())), preferred_element_type=F32)

        def gelu(zz):
            tt = zz * (zz * zz + _C0)
            return zz * jnp.tanh(tt) + zz

        ZP = o.get('zp', 0)

        def parked(v, kk):
            if kk < NK - 1 or ZP == 0:
                return v
            return jnp.concatenate([gelu(v[:ZP * 8]), v[ZP * 8:]], axis=0)

        def rev(g, kk):
            return jnp.concatenate([g[kk * 128 + j * 8:kk * 128 + j * 8 + 8] for j in reversed(range(16))], axis=0)

        def block(k, ycur, ynxt):
            r0 = k * U
            z0 = zs[0]
            z1 = zs[1]
            z2 = zs[2]
            src = xbuf.at[k % NXB]
            ocur = obuf.at[k % NOB]
            onxt = obuf.at[(k + 1) % NOB]
            wd = xf.at[pl.ds(z0, RING + 4)]
            ybd = ycur.at[pl.ds(z0, U + 1)]
            rbase = (k % 4) * U + 1

            def ring(r):
                return (rbase + r + 1) & (RING - 1)

            ev = []
            st = dict(n=0, s1=None, s2=None, z=None, up=LA, nup=0, out=[])
            evr = []
            ev2 = []
            vals = {}

            def token(T, wide=False, side=False):
                c = [e for e in ev if e[0] <= T + 1e-6]
                if o.get('notok', 0):
                    return None
                if side:
                    late = max([e[0] for e in c], default=-99)
                    c += [e for e in ev2 if late + 1.0 < e[0] <= T + 1e-6]
                if not c:
                    return None
                _, a, j = max(c, key=lambda e: e[0])
                return a[j * 8:j * 8 + 8, 0:256].astype(BF16) if wide else a[j * 8:j * 8 + 8, 0:128]

            def xtok(v, T=None):
                c = [e for e in evr if T is not None and T - o.get('rwin', 2) <= e[0] <= T]
                if c:
                    for e in c:
                        xf[RING + 3 + z2, 0:8, 384:512] = e[1]
                        evr.remove(e)
                    if not o.get('both', 0):
                        return
                xf[RING + 3 + z2, 0:8, 384:512] = v

            def conv_next(v_, T=None):
                v, n = divmod(st['n'], NCG)
                if st['n'] >= U * NCG * (1 + o.get('half', 0)):
                    return
                if v_ is not None:
                    xtok(v_, T)
                if o.get('half', 0):
                    v, n, part = st['n'] // 24, (st['n'] % 24) // 2, st['n'] % 2
                    assert v + U + 1 < st['up'], (v, st['up'])
                    cs = slice(n * 8, n * 8 + 8)
                    ts = slice(part * HW, part * HW + HW)
                    z = direct_front(n, [xf[ring(v + U - 1 + q), cs, ts] for q in range(3)], wd)
                    st['z'] = [None, [None, None, z[1][1]]]
                    zz_ = st['zk'] if part else [[], [], []]
                    zz_[0] += [pltpu.roll(a, 1, 1) for a in z[0]]
                    zz_[1] += z[1]
                    zz_[2] += [pltpu.roll(a, 127, 1) for a in z[2]]
                    st['zk'] = zz_
                    if part == 0:
                        st['y0'] = shift_sum(zz_[1], zz_[0], zz_[2], 0)
                    else:
                        finish(v, n, [st['y0']] + [shift_sum(zz_[1], zz_[0], zz_[2], t) for t in range(1, NT)], 0)
                elif WINO:
                    v, n, part = 2 * (st['n'] // 24), (st['n'] % 24) // 2, st['n'] % 2
                    assert v + U + 2 < st['up'], (v, st['up'])
                    cs = slice(n * 8, n * 8 + 8)
                    ts = slice(part * HW, part * HW + HW)
                    z = wino_front(n, [xf[ring(v + U - 1 + q), cs, ts] for q in range(4)], wd)
                    st['z'] = [None, [None, None, z[1][1][1]]]
                    zz_ = st['zk'] if part else [[[], [], []], [[], [], []]]
                    for q in range(2):
                        zz_[q][0] += [pltpu.roll(a, 1, 1) for a in z[q][0]]
                        zz_[q][1] += z[q][1]
                        zz_[q][2] += [pltpu.roll(a, 127, 1) for a in z[q][2]]
                    st['zk'] = zz_
                    if part == 0:
                        st['y0'] = [shift_sum(zz_[q][1], zz_[q][0], zz_[q][2], 0) for q in range(2)]
                    else:
                        for q in range(2):
                            y = [st['y0'][q]] + [shift_sum(zz_[q][1], zz_[q][0], zz_[q][2], t) for t in range(1, NT)]
                            finish(v + q, n, y, q)
                else:
                    assert v + U + 1 < st['up'], (v, st['up'])
                    cs = slice(n * 8, n * 8 + 8)
                    y, st['z'] = conv_piece(n, xf[ring(v + U - 1), cs, :], xf[ring(v + U), cs, :], xf[ring(v + U + 1), cs, :], wd, True)
                    finish(v, n, y, 0)
                    if T is not None:
                        ev2.append((T + o.get('zdt', 2), st['z'][1][3], 0))
                        ev2.append((T + o.get('ydt', 5), y[3], 0))
                st['n'] += 1

            def finish(v, n, y, q):
                ynxt[v, n * 8:n * 8 + 8, :] = jnp.concatenate(y, axis=1)
                if n == 0:
                    st['s1', q], st['s2', q] = y, [b * b for b in y]
                else:
                    if not o.get('hack4', 0): st['s1', q] = [a + b for a, b in zip(st['s1', q], y)]
                    if not o.get('hack3', 0): st['s2', q] = [a + b * b for a, b in zip(st['s2', q], y)]
                if n == NCG - 1:
                    ynxt[U, (v % 12) * 8:(v % 12) * 8 + 8, 128 + 128 * (v // 12):256 + 128 * (v // 12)] = rstd4(st['s1', q], st['s2', q])

            def run(T, kind, u, h, n):
                if kind == 'c':
                    v = token(T)
                    conv_next(v if v is not None or st['z'] is None or o.get('notok', 0) else st['z'][1][2], T)
                elif kind == 'z':
                    conv_next(None if st['z'] is None else st['z'][1][2])
                elif kind == 'up':
                    c = [e for e in st['out'] if T - o.get('uwin', 0) <= e[0] <= T]
                    v = c[-1][1] if c else None if o.get('upfree', 0) and T > 8 else token(T, True)
                    if v is not None:
                        xbuf[NXB + z1, 0, 0:8, 0:256] = v
                    cs = slice(n * (C // NUP), (n + 1) * (C // NUP))
                    xf[ring(st['up']), cs, :] = src[u, cs, :].astype(F32)
                    st['nup'] += 1
                    if n == NUP - 1:
                        st['up'] += 1
                elif kind == 'ld':
                    v = token(T)
                    if v is not None:
                        ycur[U + z1, 0:8, 0:128] = v
                    if ('rs', u) not in vals:
                        vals['rs', u] = ybd[U, (u % 12) * 8:(u % 12) * 8 + 8, 128 + 128 * (u // 12):256 + 128 * (u // 12)]
                    t = 2 * h + n
                    vals['h', u, t] = ybd[u, :, t * 128:(t + 1) * 128] * pick(vals['rs', u], t)
                elif kind == 'w1':
                    v = token(T, side=o.get('side', 0))
                    if v is not None:
                        w1s[1 + z1, 0:8, :] = pltpu.bitcast(v, U32)
                    a0, a1 = n
                    vals.setdefault(('w1', u, h), []).append(w1s[z0, a0 * 8:a1 * 8, :])
                elif kind == 'w2':
                    v = token(T)
                    if v is not None:
                        w2s[NK + z1, 0:8, :] = pltpu.bitcast(v, U32)
                    vals['w2', u, h, n] = w2s[n + z0]
                elif kind == 'gl':
                    v = token(T)
                    if v is not None:
                        gs[E + z1 * 8:E + z1 * 8 + 8, 0:128] = v
                    vals['g', u, h, n] = parked(gs[pl.ds(pl.multiple_of(z0 * 8 + n * 128, 8), 128), :], n)
                elif kind == 'gp':
                    m = (n // 16) * 16 + 15 - n % 16
                    gs[m * 8:m * 8 + 8, :] = vals['graw' if n < 48 - o.get('zp', 0) else 'zraw'][n * 8:n * 8 + 8, :]
                elif kind == 'pk':
                    kk, q = n
                    nr = C // NRP
                    rs8 = slice(q * nr, q * nr + nr)
                    P = vals['P', u, h]
                    if MODE == 3:
                        accx[2 * h + kk + z1, rs8, :] = P[kk][rs8]
                    elif MODE == 5:
                        if kk == 0:
                            accx[2 * h + z1, rs8, :] = P[0][rs8]
                    elif MODE == 0:
                        pass
                    elif kk == 1:
                        accx[2 * h + z1, rs8, :] = P[0][rs8] + P[1][rs8]
                elif kind == 'r':
                    v = token(T)
                    if v is not None:
                        if not o.get('noxf', 0):
                            xtok(v)
                        if MODE != 0:
                            accx[4 + z1, 0:8, 0:128] = v
                    nr = C // NRP
                    rs8 = slice(n * nr, n * nr + nr)
                    hs = slice(h * HW, h * HW + HW)
                    gbv = wtap(wd, 12, rs8)
                    res = xf[ring(u), rs8, hs] + jnp.concatenate([gbv, gbv], axis=1)
                    P = vals['P', u, h]
                    if MODE == 0:
                        a = (P[0][rs8] + P[1][rs8]) + res
                        if o.get('hack2', 0):
                            a = (P[0][rs8] + P[1][rs8])
                    elif MODE == 5:
                        a = (accx[2 * h + z0, rs8, :] + res) + P[1][rs8]
                    else:
                        a = accx[2 * h + z0, rs8, :] + res
                    if MODE == 3:
                        a = a + accx[2 * h + 1 + z0, rs8, :]
                    outf = a + vals['P', u, h][2][rs8]
                    if o.get('assoc', 0) == 1:
                        outf = ((P[0][rs8] + P[1][rs8]) + P[2][rs8]) + res
                    elif o.get('assoc', 0) == 2:
                        outf = (P[0][rs8] + P[1][rs8]) + (P[2][rs8] + res)
                    elif o.get('assoc', 0) == 3:
                        outf = ((res + P[0][rs8]) + P[1][rs8]) + P[2][rs8]
                    elif o.get('assoc', 0) == 4:
                        outf = (P[0][rs8] + (P[1][rs8] + res)) + P[2][rs8]
                    out = outf.astype(o_hbm.dtype)
                    st['out'].append((T, out[nr - 8:nr, :]))
                    if o.get('rtok', 0):
                        for t_ in range(o['rtok']):
                            evr.append((T + 0.02, outf[nr - 8 * (1 + t_ // 2):, 128 * (1 - t_ % 2):][0:8, 0:128]))
                    if u + 1 < U:
                        ocur[u + 1, rs8, hs] = out
                    else:
                        onxt[0, rs8, hs] = out

            S0 = ((0.0, 0.0), (18.0, 0.0))
            items = []
            w1items = {}
            add = lambda T, kind, u, h, n: items.append((T, len(items), kind, u, h, n))
            for e in range(o.get('early', 0)):
                add(o['et'][e] if 'et' in o else -20 + e, 'z', 0, 0, 0)
            m2start = lambda u, h: 42 * u + (24 if h == 0 else 42)
            for u in range(-1, U):
                if u >= 0:
                    for j, tau in enumerate(o.get('cf' if u == 0 else 'cl' if u == U - 1 else 'c', o['c'])):
                        if (u, j) not in o.get('skip', ()):
                            add(42 * u + tau, 'c', u, 0, 0)
                    for n in range(NUP):
                        add(42 * u + o.get('upf' if u == 0 else 'up', o['up'])[n], 'up', u, 0, n)
                for h in range(2):
                    if u >= 0:
                        m1 = 42 * u + S0[h][0]
                        for n in range(2):
                            add(m1 - (o['ld'] if h == 0 else o.get('ldb', o['ld']))[n], 'ld', u, h, n)
                        a0 = 0
                        for nst, dt in (o['w1c'] if h == 0 else o.get('w1b', o['w1c'])):
                            w1items.setdefault((u, h), []).append((m1 + a0 - dt, 'w1', u, h, (a0, a0 + nst)))
                            a0 += nst
                    if (u == U - 1 and h == 1):
                        for j in range(48):
                            add(42 * u + 27 + j / 2, 'gp', u, h, j)
                        continue
                    if (u == -1 and h == 0):
                        continue
                    m2 = m2start(u, h)
                    w = 6.0 / NRP
                    for kk in range(NK):
                        add(m2 + 6 * kk - (o['w2dt'][3 * h + kk] if isinstance(o['w2dt'], tuple) else o['w2dt']), 'w2', u, h, kk)
                        if u == -1:
                            add(m2 + 6 * kk - o.get('gldt', (6, 6, 6))[kk], 'gl', u, h, kk)
                        if kk < 2:
                            for q in range(NRP):
                                add(m2 + 8 + 6 * kk + (q + 1) * w - 0.5, 'pk', u, h, (kk, q))
                    for q in range(NRP):
                        add(m2 + 20 + q * w + (o['roff'][h] if isinstance(o['roff'], tuple) else o['roff']) + o.get('rgap', 0) * q, 'r', u, h, q)
            items.sort()
            ptr = [0]

            def flush(pred):
                last = max([i_ for i_, it in enumerate(items) if pred(it)], default=-1)
                while ptr[0] <= last:
                    T, _, kind, u, h, n = items[ptr[0]]
                    run(T, kind, u, h, n)
                    ptr[0] += 1

            def mat1(u, h):
                flush(lambda it: (it[2] == 'ld' and it[3] == u and it[4] == h) or (o.get('side', 0) and it[2] == 'c' and it[0] < 42 * u + S0[h][0] + (8 if h == 0 else 5)))
                for it in w1items[u, h]:
                    run(*it)
                lhs = jnp.concatenate(vals['w1', u, h], axis=0)
                if o.get('hack1', 0):
                    lhs = jnp.concatenate([lhs[0:48]] * 4, axis=0)
                rhs = jnp.concatenate([vals['h', u, 2 * h], vals['h', u, 2 * h + 1]], axis=1)
                zz = mm(pltpu.bitcast(lhs, BF16), aug(rhs))
                g = gelu(zz)
                vals['graw'] = g
                vals['zraw'] = zz
                for kk in range(NK):
                    vals['g', u, h, kk] = rev(g, kk)
                ev.extend((42 * u + S0[h][0] + 9 + j / 2, g, j) for j in range(48))

            def mat2(u, h):
                flush(lambda it: it[2] in ('w2', 'gl') and it[3] == u and it[4] == h)
                P = [mm(pltpu.bitcast(vals['w2', u, h, kk], BF16), vals['g', u, h, kk]) for kk in range(NK)]
                vals['P', u, h] = P
                ev.extend((m2start(u, h) + 8 + 6 * kk + j / 2 + 0.01, P[kk], j) for kk in range(NK) for j in range(12))

            for u in range(U):
                if o.get('xmid') == u:
                    flush(lambda it: it[0] < 42 * u - 8)
                    xstart(k)
                mat1(u, 0)
                mat2(u - 1, 1)
                mat1(u, 1)
                mat2(u, 0)
            flush(lambda it: True)
            assert st['n'] == U * NCG * (1 + o.get('half', 0)) and st['up'] == LA + U, st

        def xstart(k):
            pl.when(k + 2 < KP)(lambda: xchunk(k + 2).start())
            if NP:
                pl.when(k + 2 == KP)(lambda: xpart().start())

        def body(k, _):
            @pl.when(k + 2 < KP)
            def _():
                xchunk(k).wait()
                xchunk(k + 2).start()

            @pl.when(k + 2 >= KP)
            def _():
                pl.when(k < KP)(lambda: xchunk(k).wait())

                @pl.when(k == KP)
                def _():
                    if NP:
                        xpart().wait()
                    xbuf[KP % NXB, NP] = jnp.zeros((C, W), BF16)

                if NP:
                    pl.when(k + 2 == KP)(lambda: xpart().start())

            pl.when((k & 1) == 0)(lambda: block(k, ya, yb))
            pl.when((k & 1) == 1)(lambda: block(k, yb, ya))

            @pl.when(k > 2)
            def _():
                ochunk(k - 2).wait()
                ochunk(k).start()

            @pl.when(k <= 2)
            def _():
                pl.when(k == 2)(lambda: ofirst.wait())
                pl.when(k == 0)(lambda: ofirst.start())
                pl.when(k > 0)(lambda: ochunk(k).start())
            return 0

        lax.fori_loop(0, NBLK, body, 0)

        acc = xf[(H - 1 + 2) % RING, :, HW:] + jnp.concatenate([wtap(xf, 12, slice(0, C))] * 2, axis=1)
        for kk in range(NK):
            acc = acc + mm(pltpu.bitcast(w2s[kk], BF16), parked(gs[kk * 128:(kk + 1) * 128, :], kk))
        obuf[NBLK % NOB, 0, :, HW:] = acc.astype(o_hbm.dtype)
        olast.start()
        ochunk(NBLK - 2).wait()
        ochunk(NBLK - 1).wait()
        olast.wait()

    return kernel, RING


_U = 8
_SCHED = {'c': (3.08, 7.0, 9.92, 13.33, 16.75, 20.17, 24.08, 28.0, 32.42, 34.83, 38.75, 40.67), 'upfree': 1, 'up': (3.0, 4.5, 4.5, 9.0, 10.5, 12.0), 'ld': (7.5, 5.5), 'w2dt': (6, 3, 4, 4, 4, 4), 'roff': (-1, -1), 'nrp': 4, 'mode': 0, 'early': 1, 'noxf': 1, 'wino': 1, 'half': 0, 'nodma': 0, 'side': 0, 'zdt': 2, 'ydt': 5, 'rtok': 0, 'rwin': 2, 'uwin': 0, 'both': 0, 'ldb': (8.0, 5.5), 'rgap': -0.25, 'casc': 0, 'zp': 8, 'gldt': (6, 6, 6), 'cf': (3.08, 7.0, 9.92, 13.83, 15.75, 20.17, 23.08, 27.0, 31.42, 34.83, 38.25, 40.67), 'cl': (3.08, 7.0, 9.92, 13.33, 15.75, 20.17, 24.08, 28.0, 32.92, 34.83, 38.25, 39.67), 'upf': (3.0, 4.5, 4.5, 9.0, 10.5, 12.0), 'w1c': ((24, 2),)}


@jax.jit
def pallas_standalone__modern_conv_block_convnext__vision_kernel(x, dw, w1, b1, w2, b2, gamma):
    U, O, FLAGS = _U, _SCHED, (('XLA_TPU_EVENLY_DISTRIBUTE_CRITICAL_NODES', True),)
    B, H, W, C = x.shape
    E = w1.shape[1]
    xt = jnp.transpose(x[0], (0, 2, 1))
    args = (dw, w1, b1, w2.T, b2.reshape(1, C), gamma.reshape(1, C))
    kern, RING = _make(H, C, W, E, U, dict(O))
    vm = pl.BlockSpec(memory_space=pltpu.VMEM)
    out = pl.pallas_call(
        kern,
        in_specs=[pl.BlockSpec(memory_space=pl.ANY)] + [pl.BlockSpec(memory_space=pl.ANY) for a in args],
        out_specs=pl.BlockSpec(memory_space=pl.ANY),
        out_shape=jax.ShapeDtypeStruct((H, C, W), x.dtype),
        scratch_shapes=[
            pltpu.VMEM((9, U, C, W), BF16),
            pltpu.SemaphoreType.DMA((4,)),
            pltpu.SemaphoreType.DMA((4,)),
            pltpu.VMEM((2, E // 2, 128), U32),
            pltpu.VMEM((E // 128 + 1, C // 2, 128), U32),
            pltpu.VMEM((RING + 4, C, W), F32),
            pltpu.VMEM((U + 1, C, W), F32),
            pltpu.VMEM((U + 1, C, W), F32),
            pltpu.VMEM((5, C, W // 2), F32),
            pltpu.VMEM((E + 8, W // 2), F32),
            pltpu.SMEM((3,), jnp.int32),
        ] + [pltpu.VMEM(args[n].shape, args[n].dtype) for n in (1, 3, 0, 2, 4, 5)] + [pltpu.SemaphoreType.DMA((len(args),)), pltpu.VMEM(args[0].shape, args[0].dtype)],
        compiler_params=pltpu.CompilerParams(vmem_limit_bytes=96 * 1024 * 1024, flags=dict(FLAGS), disable_bounds_checks=bool(dict(O).get('nobc', 1))),
    )(xt, *args)
    return jnp.transpose(out, (0, 2, 1))[None]
```

```python
import functools
import jax
import jax.numpy as jnp
from jax import lax
import jax.experimental.pallas as pl
import jax.experimental.pallas.tpu as pltpu
import numpy as np

_K0 = float(np.sqrt(2.0 / np.pi))
_K1 = _K0 * 0.044715
_A = _K1 ** (1.0 / 3.0)
_C0 = _K0 / _A
_EPS = 1e-5
F32 = jnp.float32
BF16 = jnp.bfloat16
U32 = jnp.uint32


def _make(H, C, W, E, U, o):
    NBLK = H // U
    NT = W // 128
    NCG = C // 8
    NK = E // 128
    NUP = 6
    WINO = o.get('wino_', 0)
    NWT = 12 if WINO else 9
    XL = o.get('xl', 1) + WINO
    LA = U + 2 + XL
    RING = 4 * U
    NXB = 4
    NOB = 4
    HW = W // 2
    NRP = o.get('nrp', 4)
    MODE = o.get('mode', 3)
    assert NBLK % 2 == 0

    def low2(k):
        return k % 4 if isinstance(k, int) else k & 3

    def kernel(x_hbm, dw_hbm, w1_hbm, b1_hbm, w2t_hbm, b2_hbm, g_hbm, o_hbm,
               io, xsem, osem, w1s, w2s, xf, ya, yb, accx, gs, zs,
               w1_ref, w2t_ref, dw_ref, b1_ref, b2_ref, g_ref, psem, pad):

        xbuf = io.at[pl.ds(0, 5)]
        obuf = io.at[pl.ds(5, 4)]

        def xchunk(k):
            s_ = low2(k)
            return pltpu.make_async_copy(x_hbm.at[pl.ds(k * U + LA, U)], xbuf.at[s_], xsem.at[s_])

        KP = (H - LA) // U
        NP = H - LA - KP * U

        def xpart():
            return pltpu.make_async_copy(x_hbm.at[pl.ds(H - NP, NP)], xbuf.at[KP % NXB, pl.ds(0, NP)], xsem.at[KP % NXB])

        def ochunk(k):
            s_ = low2(k)
            return pltpu.make_async_copy(obuf.at[s_], o_hbm.at[pl.ds(k * U - 1, U)], osem.at[s_])

        ofirst = pltpu.make_async_copy(obuf.at[0, pl.ds(1, U - 1)], o_hbm.at[pl.ds(0, U - 1)], osem.at[0])
        olast = pltpu.make_async_copy(obuf.at[NBLK % NOB, pl.ds(0, 1)], o_hbm.at[pl.ds(H - 1, 1)], osem.at[NBLK % NOB])

        def tiles(v):
            return [v[:, t * 128:(t + 1) * 128] for t in range(NT)]

        def wtap(ref, k, cs):
            return ref[RING + k // 4, cs, (k % 4) * 128:(k % 4) * 128 + 128]

        def conv_piece(cg, x0, x1, x2, wref, want_z=False, wino=False):
            lane = lax.broadcasted_iota(jnp.int32, (8, 128), 1)
            cs = slice(cg * 8, cg * 8 + 8)
            wv = [wtap(wref, k, cs) for k in range(9)]
            x0, x1, x2 = tiles(x0), tiles(x1), tiles(x2)
            z = [[x0[t] * wv[b] + x1[t] * wv[3 + b] + x2[t] * wv[6 + b] for t in range(NT)] for b in range(3)]
            if o.get('casc', 0):
                L1 = [pltpu.roll(v, 127, 1) for v in z[1]]
                L2 = [pltpu.roll(v, 127, 1) for v in z[2]]
                bb = [z[0][t] + jnp.where(lane == 127, L1[t + 1] if t < NT - 1 else 0.0, L1[t]) for t in range(NT)]
                Rb = [pltpu.roll(v, 1, 1) for v in bb]
                out = [jnp.where(lane == 0, Rb[t - 1] if t > 0 else z[1][0], Rb[t])
                       + jnp.where(lane == 127, L2[t + 1] if t < NT - 1 else 0.0, L2[t]) for t in range(NT)]
            else:
                Rr = [pltpu.roll(v, 1, 1) for v in z[0]]
                Ll = [pltpu.roll(v, 127, 1) for v in z[2]]
                out = []
                for t in range(NT):
                    lt = jnp.where(lane == 0, Rr[t - 1] if t > 0 else 0.0, Rr[t])
                    rt = jnp.where(lane == 127, Ll[t + 1] if t < NT - 1 else 0.0, Ll[t])
                    out.append(z[1][t] + lt + rt)
            return (out, z) if want_z else out

        def direct_front(cg, d, wref):
            cs = slice(cg * 8, cg * 8 + 8)
            wv = [wtap(wref, k, cs) for k in range(9)]
            n = d[0].shape[1] // 128
            d = [[v[:, t * 128:(t + 1) * 128] for t in range(n)] for v in d]
            return [[d[0][t] * wv[b] + d[1][t] * wv[3 + b] + d[2][t] * wv[6 + b] for t in range(n)] for b in range(3)]

        def wino_front(cg, d, wref):
            cs = slice(cg * 8, cg * 8 + 8)
            wv = [wtap(wref, k, cs) for k in range(12)]
            n = d[0].shape[1] // 128
            d = [[v[:, t * 128:(t + 1) * 128] for t in range(n)] for v in d]
            T = [(d[0][t] - d[2][t], d[1][t] + d[2][t], d[2][t] - d[1][t], d[1][t] - d[3][t]) for t in range(n)]
            z = [[[], [], []], [[], [], []]]
            for b in range(3):
                for t in range(n):
                    m0, m1, m2, m3 = (T[t][k] * wv[k * 3 + b] for k in range(4))
                    z[0][b].append(m0 + m1 + m2)
                    z[1][b].append(m1 - m2 - m3)
            return z

        def shift_sum(z1, Rr, Ll, t):
            lane = lax.broadcasted_iota(jnp.int32, (8, 128), 1)
            lt = jnp.where(lane == 0, Rr[t - 1] if t > 0 else 0.0, Rr[t])
            rt = jnp.where(lane == 127, Ll[t + 1] if t < NT - 1 else 0.0, Ll[t])
            return z1[t] + lt + rt

        def fold4(v):
            s = lax.broadcasted_iota(jnp.int32, (8, 128), 0)
            m4 = s < 4
            m2 = (s & 2) == 0
            a = jnp.where(m4, v[0], v[1]) + pltpu.roll(jnp.where(m4, v[1], v[0]), 4, 0)
            b = jnp.where(m4, v[2], v[3]) + pltpu.roll(jnp.where(m4, v[3], v[2]), 4, 0)
            w = jnp.where(m2, a + pltpu.roll(a, 6, 0), b + pltpu.roll(b, 2, 0))
            return w + pltpu.roll(w, 7, 0)

        def rstd4(s1, s2):
            m = fold4(s1) * (1.0 / C)
            q = fold4(s2) * (1.0 / C)
            return lax.rsqrt(jnp.maximum(q - m * m, 0.0) + _EPS)

        def pick(rs, t):
            sl = (0, 4, 2, 6)[t]
            return rs[sl:sl + 1, :]

        def aug(hn):
            n = hn.shape[1]
            r8 = lax.broadcasted_iota(jnp.int32, (8, n), 0)
            ones = jnp.where(r8 < 2, 1.0, 0.0).astype(F32)
            return jnp.concatenate([hn, ones, jnp.zeros((128 - C - 8, n), F32)], axis=0)

        zs[0] = 0
        zs[1] = 0
        zs[2] = 0
        LX = LA - U
        HA = o.get('ha', U)
        head = pltpu.make_async_copy(x_hbm.at[pl.ds(0, HA)], xbuf.at[NXB - 1, pl.ds(0, HA)], xsem.at[NXB - 1])
        head1 = pltpu.make_async_copy(x_hbm.at[pl.ds(HA, max(U - HA, 1))], xbuf.at[NXB - 1, pl.ds(min(HA, U - 1), max(U - HA, 1))], xsem.at[NXB - 2])
        head2 = pltpu.make_async_copy(x_hbm.at[pl.ds(U, LX)], obuf.at[NOB - 1, pl.ds(0, LX)], osem.at[NOB - 1])
        params = [pltpu.make_async_copy(a, b, psem.at[n]) for n, (a, b) in enumerate(
            [(dw_hbm, dw_ref), (w1_hbm, w1_ref), (b1_hbm, b1_ref), (w2t_hbm, w2t_ref), (b2_hbm, b2_ref), (g_hbm, g_ref)])]
        for c in params:
            c.start()
        head.start()
        if HA == U:
            head2.start()
        gs[...] = jnp.zeros(gs.shape, F32)
        xf[0] = jnp.zeros((C, W), F32)
        xf[1] = jnp.zeros((C, W), F32)
        for c in (params[0], params[4], params[5]):
            c.wait()
        if HA < U:
            head1.start()
            head2.start()
        pad[...] = dw_ref[...]
        rows = [(pad if o.get('pad', 1) and a == 0 else dw_ref)[a, b:b + 1, :].astype(F32) for a in range(3) for b in range(3)]
        plain = list(rows)
        if WINO:
            g0, g1, g2 = rows[0:3], rows[3:6], rows[6:9]
            rows = g0 + [(a + b + c) * 0.5 for a, b, c in zip(g0, g1, g2)] + [(a - b + c) * 0.5 for a, b, c in zip(g0, g1, g2)] + g2
        rows.append(b2_ref[...].astype(F32))
        rows.append(g_ref[...].astype(F32))
        p = jnp.concatenate(rows + [jnp.zeros((128 - len(rows), C), F32)], axis=0)
        p = jnp.concatenate([p, jnp.zeros((128, 128 - C), F32)], axis=1)
        pt = p.T
        for k in range(NWT):
            xf[RING + k // 4, :, (k % 4) * 128:(k % 4) * 128 + 128] = jnp.broadcast_to(pt[:C, k:k + 1], (C, 128))
        gcol = pt[:C, NWT + 1:NWT + 2]
        xf[RING + 3, :, 0:128] = jnp.broadcast_to(pt[:C, NWT:NWT + 1] * gcol, (C, 128))
        def prep_matrices():
            params[1].wait()
            params[2].wait()
            params[3].wait()
            w2f = (w2t_ref[...].astype(F32) * (gcol * (0.5 / _A))).astype(BF16)
            for k in range(NK):
                w2s[k] = pltpu.bitcast(w2f[:, k * 128:(k + 1) * 128], U32)
            w1 = w1_ref[...].astype(F32)
            w1c = (w1 - jnp.mean(w1, axis=0, keepdims=True)) * _A
            b1 = b1_ref[...].astype(F32).reshape(1, E) * _A
            b1h = b1.astype(BF16).astype(F32)
            b1l = b1 - b1h
            r8 = lax.broadcasted_iota(jnp.int32, (8, E), 0)
            tail = jnp.where(r8 == 0, b1h, jnp.where(r8 == 1, b1l, 0.0))
            waug = jnp.concatenate([w1c, tail, jnp.zeros((128 - C - 8, E), F32)], axis=0)
            wt = waug.T
            wt = jnp.concatenate([wt[kk * 128 + j * 8:kk * 128 + j * 8 + 8] for kk in range(NK) for j in reversed(range(16))], axis=0)
            w1s[0] = pltpu.bitcast(wt.astype(BF16), U32)

        if o.get('prep', 0) == 0:
            prep_matrices()
        head.wait()
        if HA == U:
            head2.wait()
            xchunk(0).start()
            xchunk(1).start()
            if o.get('xin', 1):
                xchunk(2).start()
        PR = o.get('pr', U)
        s1 = {}
        s2 = {}
        waited = []
        index0 = lambda a, b: 0
        for r0_ in range(0, U, PR):
            if HA < U and r0_ <= HA < r0_ + PR + 1 + (0 if index0(r0_, HA) else 0) and not waited:
                head1.wait()
                head2.wait()
                xchunk(0).start()
                xchunk(1).start()
                if o.get('xin', 1):
                    xchunk(2).start()
                waited.append(1)
            if o.get('prep', 0) == r0_ + 1:
                prep_matrices()
            for cg in range(NCG):
                cs = slice(cg * 8, cg * 8 + 8)

                def row(r):
                    if r < 0:
                        return jnp.zeros((8, W), F32)
                    v = (xbuf[NXB - 1, r, cs, :] if r < U else obuf[NOB - 1, r - U, cs, :]).astype(F32)
                    xf[r + 2, cs, :] = v
                    return v
                xs = {r: row(r) for r in range(r0_ - 1, r0_ + PR + 1)}
                if r0_ + PR == U:
                    for r in range(U + 1, LA):
                        row(r)
                for r in range(r0_, r0_ + PR):
                    y = conv_piece(cg, xs[r - 1], xs[r], xs[r + 1], xf)
                    ya[r, cs, :] = jnp.concatenate(y, axis=1)
                    s1[r] = y if cg == 0 else [a + b for a, b in zip(s1[r], y)]
                    s2[r] = [b * b if cg == 0 else a + b * b for a, b in zip(s2.get(r, y), y)]
            for r in range(r0_, r0_ + PR):
                ya[U, (r % 12) * 8:(r % 12) * 8 + 8, 128 + 128 * (r // 12):256 + 128 * (r // 12)] = rstd4(s1[r], s2[r])

        mm = lambda a, b: lax.dot_general(a, b, (((1,), (0,)), ((), ())), preferred_element_type=F32)

        def gelu(zz):
            tt = zz * (zz * zz + _C0)
            return zz * jnp.tanh(tt) + zz

        ZP = o.get('zp', 0)

        def parked(v, kk):
            if kk < NK - 1 or ZP == 0:
                return v
            return jnp.concatenate([gelu(v[:ZP * 8]), v[ZP * 8:]], axis=0)

        def rev(g, kk):
            return jnp.concatenate([g[kk * 128 + j * 8:kk * 128 + j * 8 + 8] for j in reversed(range(16))], axis=0)

        def block(k, ycur, ynxt):
            r0 = k * U
            z0 = zs[0]
            z1 = zs[1]
            z2 = zs[2]
            src = xbuf.at[k % NXB]
            ocur = obuf.at[k % NOB]
            onxt = obuf.at[(k + 1) % NOB]
            wd = xf.at[pl.ds(z0, RING + 4)]
            ybd = ycur.at[pl.ds(z0, U + 1)]
            rbase = (k % 4) * U + 1

            def ring(r):
                return (rbase + r + 1) & (RING - 1)

            ev = []
            st = dict(n=0, s1=None, s2=None, z=None, up=LA, nup=0, out=[])
            evr = []
            ev2 = []
            vals = {}

            def token(T, wide=False, side=False):
                c = [e for e in ev if e[0] <= T + 1e-6]
                if o.get('notok', 0):
                    return None
                if side:
                    late = max([e[0] for e in c], default=-99)
                    c += [e for e in ev2 if late + 1.0 < e[0] <= T + 1e-6]
                if not c:
                    return None
                _, a, j = max(c, key=lambda e: e[0])
                return a[j * 8:j * 8 + 8, 0:256].astype(BF16) if wide else a[j * 8:j * 8 + 8, 0:128]

            def xtok(v, T=None):
                c = [e for e in evr if T is not None and T - o.get('rwin', 2) <= e[0] <= T]
                if c:
                    for e in c:
                        xf[RING + 3 + z2, 0:8, 384:512] = e[1]
                        evr.remove(e)
                    if not o.get('both', 0):
                        return
                xf[RING + 3 + z2, 0:8, 384:512] = v

            def conv_next(v_, T=None):
                v, n = divmod(st['n'], NCG)
                if st['n'] >= U * NCG * (1 + o.get('half', 0)):
                    return
                if v_ is not None:
                    xtok(v_, T)
                if o.get('half', 0):
                    v, n, part = st['n'] // 24, (st['n'] % 24) // 2, st['n'] % 2
                    assert v + U + 1 < st['up'], (v, st['up'])
                    cs = slice(n * 8, n * 8 + 8)
                    ts = slice(part * HW, part * HW + HW)
                    z = direct_front(n, [xf[ring(v + U - 1 + q), cs, ts] for q in range(3)], wd)
                    st['z'] = [None, [None, None, z[1][1]]]
                    zz_ = st['zk'] if part else [[], [], []]
                    zz_[0] += [pltpu.roll(a, 1, 1) for a in z[0]]
                    zz_[1] += z[1]
                    zz_[2] += [pltpu.roll(a, 127, 1) for a in z[2]]
                    st['zk'] = zz_
                    if part == 0:
                        st['y0'] = shift_sum(zz_[1], zz_[0], zz_[2], 0)
                    else:
                        finish(v, n, [st['y0']] + [shift_sum(zz_[1], zz_[0], zz_[2], t) for t in range(1, NT)], 0)
                elif WINO:
                    v, n, part = 2 * (st['n'] // 24), (st['n'] % 24) // 2, st['n'] % 2
                    assert v + U + 2 < st['up'], (v, st['up'])
                    cs = slice(n * 8, n * 8 + 8)
                    ts = slice(part * HW, part * HW + HW)
                    z = wino_front(n, [xf[ring(v + U - 1 + q), cs, ts] for q in range(4)], wd)
                    st['z'] = [None, [None, None, z[1][1][1]]]
                    zz_ = st['zk'] if part else [[[], [], []], [[], [], []]]
                    for q in range(2):
                        zz_[q][0] += [pltpu.roll(a, 1, 1) for a in z[q][0]]
                        zz_[q][1] += z[q][1]
                        zz_[q][2] += [pltpu.roll(a, 127, 1) for a in z[q][2]]
                    st['zk'] = zz_
                    if part == 0:
                        st['y0'] = [shift_sum(zz_[q][1], zz_[q][0], zz_[q][2], 0) for q in range(2)]
                    else:
                        for q in range(2):
                            y = [st['y0'][q]] + [shift_sum(zz_[q][1], zz_[q][0], zz_[q][2], t) for t in range(1, NT)]
                            finish(v + q, n, y, q)
                else:
                    assert v + U + 1 < st['up'], (v, st['up'])
                    cs = slice(n * 8, n * 8 + 8)
                    y, st['z'] = conv_piece(n, xf[ring(v + U - 1), cs, :], xf[ring(v + U), cs, :], xf[ring(v + U + 1), cs, :], wd, True)
                    finish(v, n, y, 0)
                    if T is not None:
                        ev2.append((T + o.get('zdt', 2), st['z'][1][3], 0))
                        ev2.append((T + o.get('ydt', 5), y[3], 0))
                st['n'] += 1

            def finish(v, n, y, q):
                ynxt[v, n * 8:n * 8 + 8, :] = jnp.concatenate(y, axis=1)
                if n == 0:
                    st['s1', q], st['s2', q] = y, [b * b for b in y]
                else:
                    if not o.get('hack4', 0): st['s1', q] = [a + b for a, b in zip(st['s1', q], y)]
                    if not o.get('hack3', 0): st['s2', q] = [a + b * b for a, b in zip(st['s2', q], y)]
                if n == NCG - 1:
                    ynxt[U, (v % 12) * 8:(v % 12) * 8 + 8, 128 + 128 * (v // 12):256 + 128 * (v // 12)] = rstd4(st['s1', q], st['s2', q])

            def run(T, kind, u, h, n):
                if kind == 'c':
                    v = token(T)
                    conv_next(v if v is not None or st['z'] is None or o.get('notok', 0) else st['z'][1][2], T)
                elif kind == 'z':
                    conv_next(None if st['z'] is None else st['z'][1][2])
                elif kind == 'up':
                    c = [e for e in st['out'] if T - o.get('uwin', 0) <= e[0] <= T]
                    v = c[-1][1] if c else None if o.get('upfree', 0) and T > 8 else token(T, True)
                    if v is not None:
                        xbuf[NXB + z1, 0, 0:8, 0:256] = v
                    cs = slice(n * (C // NUP), (n + 1) * (C // NUP))
                    xf[ring(st['up']), cs, :] = src[u, cs, :].astype(F32)
                    st['nup'] += 1
                    if n == NUP - 1:
                        st['up'] += 1
                elif kind == 'ld':
                    v = token(T)
                    if v is not None:
                        ycur[U + z1, 0:8, 0:128] = v
                    if ('rs', u) not in vals:
                        vals['rs', u] = ybd[U, (u % 12) * 8:(u % 12) * 8 + 8, 128 + 128 * (u // 12):256 + 128 * (u // 12)]
                    t = 2 * h + n
                    vals['h', u, t] = ybd[u, :, t * 128:(t + 1) * 128] * pick(vals['rs', u], t)
                elif kind == 'w1':
                    v = token(T, side=o.get('side', 0))
                    if v is not None:
                        w1s[1 + z1, 0:8, :] = pltpu.bitcast(v, U32)
                    a0, a1 = n
                    vals.setdefault(('w1', u, h), []).append(w1s[z0, a0 * 8:a1 * 8, :])
                elif kind == 'w2':
                    v = token(T)
                    if v is not None:
                        w2s[NK + z1, 0:8, :] = pltpu.bitcast(v, U32)
                    vals['w2', u, h, n] = w2s[n + z0]
                elif kind == 'gl':
                    v = token(T)
                    if v is not None:
                        gs[E + z1 * 8:E + z1 * 8 + 8, 0:128] = v
                    vals['g', u, h, n] = parked(gs[pl.ds(pl.multiple_of(z0 * 8 + n * 128, 8), 128), :], n)
                elif kind == 'gp':
                    m = (n // 16) * 16 + 15 - n % 16
                    gs[m * 8:m * 8 + 8, :] = vals['graw' if n < 48 - o.get('zp', 0) else 'zraw'][n * 8:n * 8 + 8, :]
                elif kind == 'pk':
                    kk, q = n
                    nr = C // NRP
                    rs8 = slice(q * nr, q * nr + nr)
                    P = vals['P', u, h]
                    if MODE == 3:
                        accx[2 * h + kk + z1, rs8, :] = P[kk][rs8]
                    elif MODE == 5:
                        if kk == 0:
                            accx[2 * h + z1, rs8, :] = P[0][rs8]
                    elif MODE == 0:
                        pass
                    elif kk == 1:
                        accx[2 * h + z1, rs8, :] = P[0][rs8] + P[1][rs8]
                elif kind == 'r':
                    v = token(T)
                    if v is not None:
                        if not o.get('noxf', 0):
                            xtok(v)
                        if MODE != 0:
                            accx[4 + z1, 0:8, 0:128] = v
                    nr = C // NRP
                    rs8 = slice(n * nr, n * nr + nr)
                    hs = slice(h * HW, h * HW + HW)
                    gbv = wtap(wd, 12, rs8)
                    res = xf[ring(u), rs8, hs] + jnp.concatenate([gbv, gbv], axis=1)
                    P = vals['P', u, h]
                    if MODE == 0:
                        a = (P[0][rs8] + P[1][rs8]) + res
                        if o.get('hack2', 0):
                            a = (P[0][rs8] + P[1][rs8])
                    elif MODE == 5:
                        a = (accx[2 * h + z0, rs8, :] + res) + P[1][rs8]
                    else:
                        a = accx[2 * h + z0, rs8, :] + res
                    if MODE == 3:
                        a = a + accx[2 * h + 1 + z0, rs8, :]
                    outf = a + vals['P', u, h][2][rs8]
                    if o.get('assoc', 0) == 1:
                        outf = ((P[0][rs8] + P[1][rs8]) + P[2][rs8]) + res
                    elif o.get('assoc', 0) == 2:
                        outf = (P[0][rs8] + P[1][rs8]) + (P[2][rs8] + res)
                    elif o.get('assoc', 0) == 3:
                        outf = ((res + P[0][rs8]) + P[1][rs8]) + P[2][rs8]
                    elif o.get('assoc', 0) == 4:
                        outf = (P[0][rs8] + (P[1][rs8] + res)) + P[2][rs8]
                    out = outf.astype(o_hbm.dtype)
                    st['out'].append((T, out[nr - 8:nr, :]))
                    if o.get('rtok', 0):
                        for t_ in range(o['rtok']):
                            evr.append((T + 0.02, outf[nr - 8 * (1 + t_ // 2):, 128 * (1 - t_ % 2):][0:8, 0:128]))
                    if u + 1 < U:
                        ocur[u + 1, rs8, hs] = out
                    else:
                        onxt[0, rs8, hs] = out

            S0 = ((0.0, 0.0), (18.0, 0.0))
            items = []
            w1items = {}
            add = lambda T, kind, u, h, n: items.append((T, len(items), kind, u, h, n))
            for e in range(o.get('early', 0)):
                add(o['et'][e] if 'et' in o else -20 + e, 'z', 0, 0, 0)
            m2start = lambda u, h: 42 * u + (24 if h == 0 else 42)
            for u in range(-1, U):
                if u >= 0:
                    for j, tau in enumerate(o.get('cf' if u == 0 else 'cl' if u == U - 1 else 'c', o['c'])):
                        if (u, j) not in o.get('skip', ()):
                            add(42 * u + tau, 'c', u, 0, 0)
                    for n in range(NUP):
                        add(42 * u + o.get('upf' if u == 0 else 'up', o['up'])[n], 'up', u, 0, n)
                for h in range(2):
                    if u >= 0:
                        m1 = 42 * u + S0[h][0]
                        for n in range(2):
                            add(m1 - (o['ld'] if h == 0 else o.get('ldb', o['ld']))[n], 'ld', u, h, n)
                        a0 = 0
                        for nst, dt in (o['w1c'] if h == 0 else o.get('w1b', o['w1c'])):
                            w1items.setdefault((u, h), []).append((m1 + a0 - dt, 'w1', u, h, (a0, a0 + nst)))
                            a0 += nst
                    if (u == U - 1 and h == 1):
                        for j in range(48):
                            add(42 * u + 27 + j / 2, 'gp', u, h, j)
                        continue
                    if (u == -1 and h == 0):
                        continue
                    m2 = m2start(u, h)
                    w = 6.0 / NRP
                    for kk in range(NK):
                        add(m2 + 6 * kk - (o['w2dt'][3 * h + kk] if isinstance(o['w2dt'], tuple) else o['w2dt']), 'w2', u, h, kk)
                        if u == -1:
                            add(m2 + 6 * kk - o.get('gldt', (6, 6, 6))[kk], 'gl', u, h, kk)
                        if kk < 2:
                            for q in range(NRP):
                                add(m2 + 8 + 6 * kk + (q + 1) * w - 0.5, 'pk', u, h, (kk, q))
                    for q in range(NRP):
                        add(m2 + 20 + q * w + (o['roff'][h] if isinstance(o['roff'], tuple) else o['roff']) + o.get('rgap', 0) * q, 'r', u, h, q)
            items.sort()
            ptr = [0]

            def flush(pred):
                last = max([i_ for i_, it in enumerate(items) if pred(it)], default=-1)
                while ptr[0] <= last:
                    T, _, kind, u, h, n = items[ptr[0]]
                    run(T, kind, u, h, n)
                    ptr[0] += 1

            def mat1(u, h):
                flush(lambda it: (it[2] == 'ld' and it[3] == u and it[4] == h) or (o.get('side', 0) and it[2] == 'c' and it[0] < 42 * u + S0[h][0] + (8 if h == 0 else 5)))
                for it in w1items[u, h]:
                    run(*it)
                lhs = jnp.concatenate(vals['w1', u, h], axis=0)
                if o.get('hack1', 0):
                    lhs = jnp.concatenate([lhs[0:48]] * 4, axis=0)
                rhs = jnp.concatenate([vals['h', u, 2 * h], vals['h', u, 2 * h + 1]], axis=1)
                zz = mm(pltpu.bitcast(lhs, BF16), aug(rhs))
                g = gelu(zz)
                vals['graw'] = g
                vals['zraw'] = zz
                for kk in range(NK):
                    vals['g', u, h, kk] = rev(g, kk)
                ev.extend((42 * u + S0[h][0] + 9 + j / 2, g, j) for j in range(48))

            def mat2(u, h):
                flush(lambda it: it[2] in ('w2', 'gl') and it[3] == u and it[4] == h)
                P = [mm(pltpu.bitcast(vals['w2', u, h, kk], BF16), vals['g', u, h, kk]) for kk in range(NK)]
                vals['P', u, h] = P
                ev.extend((m2start(u, h) + 8 + 6 * kk + j / 2 + 0.01, P[kk], j) for kk in range(NK) for j in range(12))

            for u in range(U):
                if o.get('xmid') == u:
                    flush(lambda it: it[0] < 42 * u - 8)
                    xstart(k)
                mat1(u, 0)
                mat2(u - 1, 1)
                mat1(u, 1)
                if u == U - 1:
                    flush(lambda it: it[2] == 'r' and it[3] == u - 1 and it[4] == 1)
                    pl.when(k == 0)(lambda: ofirst.start())
                    pl.when(k > 0)(lambda: ochunk(k).start())
                    if o.get('xin', 1):
                        pl.when(k + 3 < KP)(lambda: xchunk(k + 3).start())
                mat2(u, 0)
            flush(lambda it: True)
            assert st['n'] == U * NCG * (1 + o.get('half', 0)) and st['up'] == LA + U, st

        def xstart(k):
            pl.when(k + 2 < KP)(lambda: xchunk(k + 2).start())
            if NP:
                pl.when(k + 2 == KP)(lambda: xpart().start())

        def body(k, _):
            @pl.when(k + 2 < KP)
            def _():
                xchunk(k).wait()
                if not o.get('xin', 1):
                    xchunk(k + 2).start()

            @pl.when(k + 2 >= KP)
            def _():
                pl.when(k < KP)(lambda: xchunk(k).wait())

                @pl.when(k == KP)
                def _():
                    if NP:
                        xpart().wait()
                    xbuf[KP % NXB, NP] = jnp.zeros((C, W), BF16)

                if NP:
                    pl.when(k + 2 == KP)(lambda: xpart().start())

            pl.when((k & 1) == 0)(lambda: block(k, ya, yb))
            pl.when((k & 1) == 1)(lambda: block(k, yb, ya))

            @pl.when(k > 2)
            def _():
                ochunk(k - 2).wait()

            pl.when(k == 2)(lambda: ofirst.wait())
            return 0

        lax.fori_loop(0, NBLK, body, 0)

        acc = xf[(H - 1 + 2) % RING, :, HW:] + jnp.concatenate([wtap(xf, 12, slice(0, C))] * 2, axis=1)
        for kk in range(NK):
            acc = acc + mm(pltpu.bitcast(w2s[kk], BF16), parked(gs[kk * 128:(kk + 1) * 128, :], kk))
        obuf[NBLK % NOB, 0, :, HW:] = acc.astype(o_hbm.dtype)
        olast.start()
        ochunk(NBLK - 2).wait()
        ochunk(NBLK - 1).wait()
        olast.wait()

    return kernel, RING


_U = 16
_SCHED = {'c': (3.08, 7.0, 9.92, 13.33, 16.75, 20.17, 24.08, 28.0, 32.42, 34.83, 38.75, 40.67), 'upfree': 1, 'up': (3.0, 4.5, 4.5, 9.0, 10.5, 12.0), 'ld': (7.5, 5.5), 'w2dt': (6, 3, 4, 4, 4, 4), 'roff': (-1, -1), 'nrp': 4, 'mode': 0, 'early': 1, 'noxf': 1, 'wino': 1, 'half': 0, 'nodma': 0, 'side': 0, 'zdt': 2, 'ydt': 5, 'rtok': 0, 'rwin': 2, 'uwin': 0, 'both': 0, 'ldb': (8.0, 5.5), 'rgap': -0.25, 'casc': 0, 'zp': 8, 'gldt': (6, 6, 6), 'cf': (3.08, 7.0, 9.92, 13.83, 15.75, 20.17, 23.08, 27.0, 31.42, 34.83, 38.25, 40.67), 'cl': (3.08, 7.0, 9.92, 13.33, 15.75, 20.17, 24.08, 28.0, 32.92, 34.83, 38.25, 39.67), 'upf': (3.0, 4.5, 4.5, 9.0, 10.5, 12.0), 'ha': 5, 'pr': 4, 'prep': 1, 'xin': 0, 'w1c': ((24, 2),)}


@jax.jit
def pallas_standalone__modern_conv_block_convnext__vision_kernel(x, dw, w1, b1, w2, b2, gamma):
    U, O, FLAGS = _U, _SCHED, (('XLA_TPU_EVENLY_DISTRIBUTE_CRITICAL_NODES', True),)
    B, H, W, C = x.shape
    E = w1.shape[1]
    xt = jnp.transpose(x[0], (0, 2, 1))
    args = (dw, w1, b1, w2.T, b2.reshape(1, C), gamma.reshape(1, C))
    kern, RING = _make(H, C, W, E, U, dict(O))
    vm = pl.BlockSpec(memory_space=pltpu.VMEM)
    out = pl.pallas_call(
        kern,
        in_specs=[pl.BlockSpec(memory_space=pl.ANY)] + [pl.BlockSpec(memory_space=pl.ANY) for a in args],
        out_specs=pl.BlockSpec(memory_space=pl.ANY),
        out_shape=jax.ShapeDtypeStruct((H, C, W), x.dtype),
        scratch_shapes=[
            pltpu.VMEM((9, U, C, W), BF16),
            pltpu.SemaphoreType.DMA((4,)),
            pltpu.SemaphoreType.DMA((4,)),
            pltpu.VMEM((2, E // 2, 128), U32),
            pltpu.VMEM((E // 128 + 1, C // 2, 128), U32),
            pltpu.VMEM((RING + 4, C, W), F32),
            pltpu.VMEM((U + 1, C, W), F32),
            pltpu.VMEM((U + 1, C, W), F32),
            pltpu.VMEM((5, C, W // 2), F32),
            pltpu.VMEM((E + 8, W // 2), F32),
            pltpu.SMEM((3,), jnp.int32),
        ] + [pltpu.VMEM(args[n].shape, args[n].dtype) for n in (1, 3, 0, 2, 4, 5)] + [pltpu.SemaphoreType.DMA((len(args),)), pltpu.VMEM(args[0].shape, args[0].dtype)],
        compiler_params=pltpu.CompilerParams(vmem_limit_bytes=96 * 1024 * 1024, flags=dict(FLAGS), disable_bounds_checks=bool(dict(O).get('nobc', 1))),
    )(xt, *args)
    return jnp.transpose(out, (0, 2, 1))[None]
```

```python
import jax
import jax.numpy as jnp
from jax import lax
import jax.experimental.pallas as pl
import jax.experimental.pallas.tpu as pltpu
import numpy as np

F32 = jnp.float32
BF16 = jnp.bfloat16
U32 = jnp.uint32

_K0 = float(np.sqrt(2.0 / np.pi))
_A = (_K0 * 0.044715) ** (1.0 / 3.0)
_C0 = _K0 / _A
_EPS = 1e-5

_U = 16
_CONV = {"first": (3.08, 7.0, 9.92, 13.83, 15.75, 20.17, 23.08, 27.0, 31.42, 34.83, 38.25, 40.67),
         "mid": (3.08, 7.0, 9.92, 13.33, 16.75, 20.17, 24.08, 28.0, 32.42, 34.83, 38.75, 40.67),
         "last": (3.08, 7.0, 9.92, 13.33, 15.75, 20.17, 24.08, 28.0, 32.92, 34.83, 38.25, 39.67)}
_UNPACK = (3.0, 4.5, 4.5, 9.0, 10.5, 12.0)
_RHS_LEAD = ((7.5, 5.5), (8.0, 5.5))
_W1_LEAD = (2, 2)
_W2_LEAD = (6, 3, 4, 4, 4, 4)
_OUT_OFF, _OUT_SKEW, _OUT_PIECES = -1, -0.25, 4
_PARK_LEAD = 6
_RAW_CHUNKS = 10
_HEAD, _PRO = 5, 4


def _make_kernel(H, C, W, E):
    U = _U
    NBLK, NT, NCG, NK, HW = H // U, W // 128, C // 8, E // 128, W // 2
    NUP = len(_UNPACK)
    LA = U + 3
    RING = 4 * U
    KP = (H - LA) // U
    NP = H - LA - KP * U
    assert H % U == 0 and NBLK % 4 == 0 and NT == 4 and C == 96 and E % 128 == 0 and NP > 0 and U <= 36

    def mod4(k):
        return k % 4 if isinstance(k, int) else k & 3

    def kernel(x_hbm, dw_hbm, w1_hbm, b1_hbm, w2t_hbm, b2_hbm, g_hbm, o_hbm,
               io, xsem, osem, w1s, w2s, xf, ya, yb, gs, zs,
               w1_ref, w2t_ref, dw_ref, b1_ref, b2_ref, g_ref, psem, dw2_ref):
        xbuf = io.at[pl.ds(0, 5)]
        obuf = io.at[pl.ds(5, 4)]

        def xchunk(k):
            return pltpu.make_async_copy(x_hbm.at[pl.ds(k * U + LA, U)], xbuf.at[mod4(k)], xsem.at[mod4(k)])

        def xpart():
            return pltpu.make_async_copy(x_hbm.at[pl.ds(H - NP, NP)], xbuf.at[KP % 4, pl.ds(0, NP)], xsem.at[KP % 4])

        def ochunk(k):
            return pltpu.make_async_copy(obuf.at[mod4(k)], o_hbm.at[pl.ds(k * U - 1, U)], osem.at[mod4(k)])

        ofirst = pltpu.make_async_copy(obuf.at[0, pl.ds(1, U - 1)], o_hbm.at[pl.ds(0, U - 1)], osem.at[0])
        olast = pltpu.make_async_copy(obuf.at[NBLK % 4, pl.ds(0, 1)], o_hbm.at[pl.ds(H - 1, 1)], osem.at[NBLK % 4])

        def mm(a, b):
            return lax.dot_general(a, b, (((1,), (0,)), ((), ())), preferred_element_type=F32)

        def tap(ref, k, cs):
            return ref[RING + k // 4, cs, (k % 4) * 128:(k % 4) * 128 + 128]

        def conv(cg, rows, wref):
            lane = lax.broadcasted_iota(jnp.int32, (8, 128), 1)
            cs = slice(cg * 8, cg * 8 + 8)
            wv = [tap(wref, k, cs) for k in range(9)]
            x0, x1, x2 = [[v[:, t * 128:(t + 1) * 128] for t in range(NT)] for v in rows]
            z = [[x0[t] * wv[b] + x1[t] * wv[3 + b] + x2[t] * wv[6 + b] for t in range(NT)] for b in range(3)]
            zl = [pltpu.roll(v, 1, 1) for v in z[0]]
            zr = [pltpu.roll(v, 127, 1) for v in z[2]]
            out = []
            for t in range(NT):
                lt = jnp.where(lane == 0, zl[t - 1] if t > 0 else 0.0, zl[t])
                rt = jnp.where(lane == 127, zr[t + 1] if t < NT - 1 else 0.0, zr[t])
                out.append(z[1][t] + lt + rt)
            return out, z[1]

        def fold4(v):
            s = lax.broadcasted_iota(jnp.int32, (8, 128), 0)
            m4 = s < 4
            m2 = (s & 2) == 0
            a = jnp.where(m4, v[0], v[1]) + pltpu.roll(jnp.where(m4, v[1], v[0]), 4, 0)
            b = jnp.where(m4, v[2], v[3]) + pltpu.roll(jnp.where(m4, v[3], v[2]), 4, 0)
            w = jnp.where(m2, a + pltpu.roll(a, 6, 0), b + pltpu.roll(b, 2, 0))
            return w + pltpu.roll(w, 7, 0)

        def stats(acc, y):
            if acc is None:
                return y, [b * b for b in y]
            return [a + b for a, b in zip(acc[0], y)], [a + b * b for a, b in zip(acc[1], y)]

        def put_rstd(ref, r, acc):
            m = fold4(acc[0]) * (1.0 / C)
            q = fold4(acc[1]) * (1.0 / C)
            rs = lax.rsqrt(jnp.maximum(q - m * m, 0.0) + _EPS)
            ref[U, (r % 12) * 8:(r % 12) * 8 + 8, 128 + 128 * (r // 12):256 + 128 * (r // 12)] = rs

        def gelu(z):
            t = z * (z * z + _C0)
            return z * jnp.tanh(t) + z

        def rev(g, kk):
            return jnp.concatenate([g[kk * 128 + j * 8:kk * 128 + j * 8 + 8] for j in reversed(range(16))], axis=0)

        def parked(v, kk):
            if kk < NK - 1:
                return v
            return jnp.concatenate([gelu(v[:_RAW_CHUNKS * 8]), v[_RAW_CHUNKS * 8:]], axis=0)

        for j in range(3):
            zs[j] = 0
        head0 = pltpu.make_async_copy(x_hbm.at[pl.ds(0, _HEAD)], xbuf.at[3, pl.ds(0, _HEAD)], xsem.at[3])
        head1 = pltpu.make_async_copy(x_hbm.at[pl.ds(_HEAD, U - _HEAD)], xbuf.at[3, pl.ds(_HEAD, U - _HEAD)], xsem.at[2])
        head2 = pltpu.make_async_copy(x_hbm.at[pl.ds(U, LA - U)], obuf.at[3, pl.ds(0, LA - U)], osem.at[3])
        cdw, cw1, cb1, cw2, cb2, cg_ = [
            pltpu.make_async_copy(a, b, psem.at[n]) for n, (a, b) in enumerate(
                [(dw_hbm, dw_ref), (w1_hbm, w1_ref), (b1_hbm, b1_ref), (w2t_hbm, w2t_ref), (b2_hbm, b2_ref), (g_hbm, g_ref)])]
        for c in (cdw, cw1, cb1, cw2, cb2, cg_, head0):
            c.start()
        gs[...] = jnp.zeros(gs.shape, F32)
        xf[0] = jnp.zeros((C, W), F32)
        xf[1] = jnp.zeros((C, W), F32)
        for c in (cdw, cb2, cg_):
            c.wait()
        head1.start()
        head2.start()
        dw2_ref[...] = dw_ref[...]

        rows = [(dw2_ref if a == 0 else dw_ref)[a, b:b + 1, :].astype(F32) for a in range(3) for b in range(3)]
        rows += [b2_ref[...].astype(F32), g_ref[...].astype(F32)]
        p = jnp.concatenate(rows + [jnp.zeros((128 - len(rows), C), F32)], axis=0)
        pt = jnp.concatenate([p, jnp.zeros((128, 128 - C), F32)], axis=1).T
        for k in range(9):
            xf[RING + k // 4, :, (k % 4) * 128:(k % 4) * 128 + 128] = jnp.broadcast_to(pt[:C, k:k + 1], (C, 128))
        gcol = pt[:C, 10:11]
        xf[RING + 3, :, 0:128] = jnp.broadcast_to(pt[:C, 9:10] * gcol, (C, 128))

        head0.wait()
        for c in (cw1, cb1, cw2):
            c.wait()
        w2f = (w2t_ref[...].astype(F32) * (gcol * (0.5 / _A))).astype(BF16)
        for k in range(NK):
            w2s[k] = pltpu.bitcast(w2f[:, k * 128:(k + 1) * 128], U32)
        w1 = w1_ref[...].astype(F32)
        w1c = (w1 - jnp.mean(w1, axis=0, keepdims=True)) * _A
        b1 = b1_ref[...].astype(F32).reshape(1, E) * _A
        b1h = b1.astype(BF16).astype(F32)
        r8 = lax.broadcasted_iota(jnp.int32, (8, E), 0)
        tail = jnp.where(r8 == 0, b1h, jnp.where(r8 == 1, b1 - b1h, 0.0))
        wt = jnp.concatenate([w1c, tail, jnp.zeros((128 - C - 8, E), F32)], axis=0).T
        wt = jnp.concatenate([rev(wt, kk) for kk in range(NK)], axis=0)
        w1s[0] = pltpu.bitcast(wt.astype(BF16), U32)

        acc = {}
        for q0 in range(0, U, _PRO):
            if q0 <= _HEAD < q0 + _PRO + 1:
                head1.wait()
                head2.wait()
                xchunk(0).start()
                xchunk(1).start()
            for cgi in range(NCG):
                cs = slice(cgi * 8, cgi * 8 + 8)

                def row(r):
                    if r < 0:
                        return jnp.zeros((8, W), F32)
                    v = (xbuf[3, r, cs, :] if r < U else obuf[3, r - U, cs, :]).astype(F32)
                    xf[r + 2, cs, :] = v
                    return v
                xs = {r: row(r) for r in range(q0 - 1, q0 + _PRO + 1)}
                if q0 + _PRO == U:
                    for r in range(U + 1, LA):
                        row(r)
                for r in range(q0, q0 + _PRO):
                    y, _ = conv(cgi, [xs[r - 1], xs[r], xs[r + 1]], xf)
                    ya[r, cs, :] = jnp.concatenate(y, axis=1)
                    acc[r] = stats(acc.get(r), y)
            for r in range(q0, q0 + _PRO):
                put_rstd(ya, r, acc[r])

        def block(k, ycur, ynxt):
            r0 = k * U
            z0, z1, z2 = zs[0], zs[1], zs[2]
            src = xbuf.at[k % 4]
            ocur = obuf.at[k % 4]
            onxt = obuf.at[(k + 1) % 4]
            wd = xf.at[pl.ds(z0, RING + 4)]
            ybd = ycur.at[pl.ds(z0, U + 1)]
            rbase = (k % 4) * U + 1

            def ring(r):
                return (rbase + r + 1) & (RING - 1)

            ev = []
            st = dict(n=0, acc=None, up=LA, z=None)
            vals = {}

            def token(T, wide=False):
                c = [e for e in ev if e[0] <= T + 1e-6]
                if not c:
                    return None
                _, a, j = max(c, key=lambda e: e[0])
                return a[j * 8:j * 8 + 8, 0:256].astype(BF16) if wide else a[j * 8:j * 8 + 8, 0:128]

            def run(T, kind, u, h, n):
                if kind == "conv":
                    v, n = divmod(st["n"], NCG)
                    if v >= U:
                        return
                    assert v + U + 1 < st["up"]
                    t_ = token(T)
                    if t_ is None:
                        t_ = st["z"]
                    if t_ is not None:
                        xf[RING + 3 + z2, 0:8, 384:512] = t_
                    cs = slice(n * 8, n * 8 + 8)
                    y, zc = conv(n, [xf[ring(v + U - 1 + q), cs, :] for q in range(3)], wd)
                    st["z"] = zc[2]
                    ynxt[v, cs, :] = jnp.concatenate(y, axis=1)
                    st["acc"] = stats(st["acc"] if n else None, y)
                    if n == NCG - 1:
                        put_rstd(ynxt, v, st["acc"])
                    st["n"] += 1
                elif kind == "unpack":
                    v = token(T, True) if T <= 8 else None
                    if v is not None:
                        xbuf[4 + z1, 0, 0:8, 0:256] = v
                    cs = slice(n * (C // NUP), (n + 1) * (C // NUP))
                    xf[ring(st["up"]), cs, :] = src[u, cs, :].astype(F32)
                    if n == NUP - 1:
                        st["up"] += 1
                elif kind == "rhs":
                    v = token(T)
                    if v is not None:
                        ycur[U + z1, 0:8, 0:128] = v
                    if ("rs", u) not in vals:
                        vals["rs", u] = ybd[U, (u % 12) * 8:(u % 12) * 8 + 8, 128 + 128 * (u // 12):256 + 128 * (u // 12)]
                    t = 2 * h + n
                    sl = (0, 4, 2, 6)[t]
                    vals["h", u, t] = ybd[u, :, t * 128:(t + 1) * 128] * vals["rs", u][sl:sl + 1, :]
                elif kind == "w1":
                    v = token(T)
                    if v is not None:
                        w1s[1 + z1, 0:8, :] = pltpu.bitcast(v, U32)
                    vals["w1", u, h] = w1s[z0, 0:E // 2, :]
                elif kind == "w2":
                    v = token(T)
                    if v is not None:
                        w2s[NK + z1, 0:8, :] = pltpu.bitcast(v, U32)
                    vals["w2", u, h, n] = w2s[n + z0]
                elif kind == "load":
                    v = token(T)
                    if v is not None:
                        gs[E + z1 * 8:E + z1 * 8 + 8, 0:128] = v
                    vals["g", u, h, n] = parked(gs[pl.ds(pl.multiple_of(z0 * 8 + n * 128, 8), 128), :], n)
                elif kind == "park":
                    m = (n // 16) * 16 + 15 - n % 16
                    gs[m * 8:m * 8 + 8, :] = vals["graw" if n < 48 - _RAW_CHUNKS else "zraw"][n * 8:n * 8 + 8, :]
                elif kind == "out":
                    token(T)
                    nr = C // _OUT_PIECES
                    rs8 = slice(n * nr, n * nr + nr)
                    hs = slice(h * HW, h * HW + HW)
                    gbv = tap(wd, 12, rs8)
                    res = xf[ring(u), rs8, hs] + jnp.concatenate([gbv, gbv], axis=1)
                    P = vals["P", u, h]
                    out = (((P[0][rs8] + P[1][rs8]) + res) + P[2][rs8]).astype(o_hbm.dtype)
                    if u + 1 < U:
                        ocur[u + 1, rs8, hs] = out
                    else:
                        onxt[0, rs8, hs] = out

            items, lhs1 = [], {}

            def add(T, kind, u, h, n):
                items.append((T, len(items), kind, u, h, n))

            def m1start(u, h):
                return 42 * u + 18.0 * h

            def m2start(u, h):
                return 42 * u + (24 if h == 0 else 42)

            for u in range(-1, U):
                if u >= 0:
                    for tau in _CONV["first" if u == 0 else "last" if u == U - 1 else "mid"]:
                        add(42 * u + tau, "conv", u, 0, 0)
                    for n in range(NUP):
                        add(42 * u + _UNPACK[n], "unpack", u, 0, n)
                for h in range(2):
                    if u >= 0:
                        for n in range(2):
                            add(m1start(u, h) - _RHS_LEAD[h][n], "rhs", u, h, n)
                        lhs1[u, h] = (m1start(u, h) - _W1_LEAD[h], "w1", u, h, 0)
                    if u == U - 1 and h == 1:
                        for j in range(48):
                            add(42 * u + 27 + j / 2, "park", u, h, j)
                        continue
                    if u == -1 and h == 0:
                        continue
                    m2 = m2start(u, h)
                    for kk in range(NK):
                        add(m2 + 6 * kk - _W2_LEAD[3 * h + kk], "w2", u, h, kk)
                        if u == -1:
                            add(m2 + 6 * kk - _PARK_LEAD, "load", u, h, kk)
                    for q in range(_OUT_PIECES):
                        add(m2 + 20 + q * 6.0 / _OUT_PIECES + _OUT_OFF + _OUT_SKEW * q, "out", u, h, q)
            items.sort()
            done = [0]

            def flush(pred):
                last = max([i for i, it in enumerate(items) if pred(it)], default=-1)
                while done[0] <= last:
                    T, _, kind, u, h, n = items[done[0]]
                    run(T, kind, u, h, n)
                    done[0] += 1

            def mat1(u, h):
                flush(lambda it: it[2] == "rhs" and it[3] == u and it[4] == h)
                run(*lhs1[u, h])
                lhs = jnp.concatenate([vals["w1", u, h]], axis=0)
                hn = jnp.concatenate([vals["h", u, 2 * h], vals["h", u, 2 * h + 1]], axis=1)
                s8 = lax.broadcasted_iota(jnp.int32, (8, HW), 0)
                ones = jnp.where(s8 < 2, 1.0, 0.0).astype(F32)
                z = mm(pltpu.bitcast(lhs, BF16),
                       jnp.concatenate([hn, ones, jnp.zeros((128 - C - 8, HW), F32)], axis=0))
                g = gelu(z)
                vals["graw"], vals["zraw"] = g, z
                for kk in range(NK):
                    vals["g", u, h, kk] = rev(g, kk)
                ev.extend((m1start(u, h) + 9 + j / 2, g, j) for j in range(48))

            def mat2(u, h):
                flush(lambda it: it[2] in ("w2", "load") and it[3] == u and it[4] == h)
                P = [mm(pltpu.bitcast(vals["w2", u, h, kk], BF16), vals["g", u, h, kk]) for kk in range(NK)]
                vals["P", u, h] = P
                ev.extend((m2start(u, h) + 8 + 6 * kk + j / 2 + 0.01, P[kk], j) for kk in range(NK) for j in range(12))

            run(-20, "conv", 0, 0, 0)
            for u in range(U):
                mat1(u, 0)
                mat2(u - 1, 1)
                mat1(u, 1)
                if u == U - 1:
                    flush(lambda it: it[2] == "out" and it[3] == u - 1 and it[4] == 1)
                    pl.when(k == 0)(lambda: ofirst.start())
                    pl.when(k > 0)(lambda: ochunk(k).start())
                mat2(u, 0)
            flush(lambda it: True)
            assert st["n"] == U * NCG and st["up"] == LA + U

        def body(k, carry):
            @pl.when(k + 2 < KP)
            def _():
                xchunk(k).wait()
                xchunk(k + 2).start()

            @pl.when(k + 2 >= KP)
            def _():
                pl.when(k < KP)(lambda: xchunk(k).wait())

                @pl.when(k == KP)
                def _():
                    xpart().wait()
                    xbuf[KP % 4, NP] = jnp.zeros((C, W), BF16)

                pl.when(k + 2 == KP)(lambda: xpart().start())

            pl.when((k & 1) == 0)(lambda: block(k, ya, yb))
            pl.when((k & 1) == 1)(lambda: block(k, yb, ya))
            pl.when(k > 2)(lambda: ochunk(k - 2).wait())
            pl.when(k == 2)(lambda: ofirst.wait())
            return carry

        lax.fori_loop(0, NBLK, body, 0)

        out = xf[(H - 1 + 2) % RING, :, HW:] + jnp.concatenate([tap(xf, 12, slice(0, C))] * 2, axis=1)
        for kk in range(NK):
            out = out + mm(pltpu.bitcast(w2s[kk], BF16), parked(gs[kk * 128:(kk + 1) * 128, :], kk))
        obuf[NBLK % 4, 0, :, HW:] = out.astype(o_hbm.dtype)
        olast.start()
        ochunk(NBLK - 2).wait()
        ochunk(NBLK - 1).wait()
        olast.wait()

    scratch = [
        pltpu.VMEM((9, U, C, W), BF16),
        pltpu.SemaphoreType.DMA((4,)),
        pltpu.SemaphoreType.DMA((4,)),
        pltpu.VMEM((2, E // 2, 128), U32),
        pltpu.VMEM((NK + 1, C // 2, 128), U32),
        pltpu.VMEM((RING + 4, C, W), F32),
        pltpu.VMEM((U + 1, C, W), F32),
        pltpu.VMEM((U + 1, C, W), F32),
        pltpu.VMEM((E + 8, HW), F32),
        pltpu.SMEM((3,), jnp.int32),
    ]
    return kernel, scratch


@jax.jit
def pallas_standalone__modern_conv_block_convnext__vision_kernel(x, dw, w1, b1, w2, b2, gamma):
    B, H, W, C = x.shape
    E = w1.shape[1]
    assert B == 1 and dw.shape[:2] == (3, 3)
    xt = jnp.transpose(x[0], (0, 2, 1))
    args = (dw, w1, b1, w2.T, b2.reshape(1, C), gamma.reshape(1, C))
    kernel, scratch = _make_kernel(H, C, W, E)
    scratch += [pltpu.VMEM(args[n].shape, args[n].dtype) for n in (1, 3, 0, 2, 4, 5)]
    scratch += [pltpu.SemaphoreType.DMA((len(args),)), pltpu.VMEM(dw.shape, dw.dtype)]
    hbm = pl.BlockSpec(memory_space=pl.ANY)
    out = pl.pallas_call(
        kernel,
        in_specs=[hbm] * (1 + len(args)),
        out_specs=hbm,
        out_shape=jax.ShapeDtypeStruct((H, C, W), x.dtype),
        scratch_shapes=scratch,
        compiler_params=pltpu.CompilerParams(
            vmem_limit_bytes=96 * 1024 * 1024,
            disable_bounds_checks=True,
            flags={"XLA_TPU_EVENLY_DISTRIBUTE_CRITICAL_NODES": True},
        ),
    )(xt, *args)
    return jnp.transpose(out, (0, 2, 1))[None]
```

```python
import jax
import jax.numpy as jnp
from jax import lax
import jax.experimental.pallas as pl
import jax.experimental.pallas.tpu as pltpu
import numpy as np

F32 = jnp.float32
BF16 = jnp.bfloat16
U32 = jnp.uint32

_K0 = float(np.sqrt(2.0 / np.pi))
_A = (_K0 * 0.044715) ** (1.0 / 3.0)
_C0 = _K0 / _A
_EPS = 1e-5

_U = 16
_CONV = {"first": (3.08, 7.0, 9.92, 13.83, 15.25, 20.17, 23.08, 27.0, 31.42, 34.83, 37.75, 40.67),
         "mid": (3.08, 7.0, 9.92, 13.33, 16.75, 20.17, 24.08, 28.0, 32.42, 34.83, 38.75, 41.17),
         "last": (3.08, 7.0, 9.92, 13.33, 15.75, 20.17, 24.08, 28.0, 32.92, 34.83, 38.25, 39.67)}
_UNPACK = (4.0, 4.5, 4.5, 10.5, 10.5, 12.0)
_RHS_LEAD = ((7.5, 5.5), (7.0, 5.5))
_W1_LEAD = (6, 2)
_W2_LEAD = (6, 3, 4, 4, 4, 4)
_OUT_OFF, _OUT_SKEW, _OUT_PIECES = -1, -0.25, 4
_PARK_LEAD = 6
_RAW_CHUNKS = 10
_HEAD, _PRO = 5, 4


def _make_kernel(H, C, W, E):
    U = _U
    NBLK, NT, NCG, NK, HW = H // U, W // 128, C // 8, E // 128, W // 2
    NUP = len(_UNPACK)
    LA = U + 3
    RING = 2 * U
    KP = (H - LA) // U
    NP = H - LA - KP * U
    assert H % U == 0 and NBLK % 4 == 0 and NT == 4 and C == 96 and E % 128 == 0 and NP > 0 and U <= 36

    def mod4(k):
        return k % 4 if isinstance(k, int) else k & 3

    def kernel(x_hbm, dw_hbm, w1_hbm, b1_hbm, w2t_hbm, b2_hbm, g_hbm, o_hbm,
               io, xsem, osem, w1s, w2s, xf, xr, ya, yb, gs, zs,
               w1_ref, w2t_ref, dw_ref, b1_ref, b2_ref, g_ref, psem, dw2_ref):
        xbuf = io.at[pl.ds(0, 5)]
        obuf = io.at[pl.ds(5, 4)]

        def xchunk(k):
            return pltpu.make_async_copy(x_hbm.at[pl.ds(k * U + LA, U)], xbuf.at[mod4(k)], xsem.at[mod4(k)])

        def xpart():
            return pltpu.make_async_copy(x_hbm.at[pl.ds(H - NP, NP)], xbuf.at[KP % 4, pl.ds(0, NP)], xsem.at[KP % 4])

        def ochunk(k):
            return pltpu.make_async_copy(obuf.at[mod4(k)], o_hbm.at[pl.ds(k * U - 1, U)], osem.at[mod4(k)])

        ofirst = pltpu.make_async_copy(obuf.at[0, pl.ds(1, U - 1)], o_hbm.at[pl.ds(0, U - 1)], osem.at[0])
        olast = pltpu.make_async_copy(obuf.at[NBLK % 4, pl.ds(0, 1)], o_hbm.at[pl.ds(H - 1, 1)], osem.at[NBLK % 4])

        def mm(a, b):
            return lax.dot_general(a, b, (((1,), (0,)), ((), ())), preferred_element_type=F32)

        def tap(ref, k, cs):
            return ref[k // 4, cs, (k % 4) * 128:(k % 4) * 128 + 128]

        def conv(cg, rows, wref):
            lane = lax.broadcasted_iota(jnp.int32, (8, 128), 1)
            cs = slice(cg * 8, cg * 8 + 8)
            wv = [tap(wref, k, cs) for k in range(9)]
            x0, x1, x2 = [[v[:, t * 128:(t + 1) * 128] for t in range(NT)] for v in rows]
            z = [[x0[t] * wv[b] + x1[t] * wv[3 + b] + x2[t] * wv[6 + b] for t in range(NT)] for b in range(3)]
            zl = [pltpu.roll(v, 1, 1) for v in z[0]]
            zr = [pltpu.roll(v, 127, 1) for v in z[2]]
            out = []
            for t in range(NT):
                lt = jnp.where(lane == 0, zl[t - 1] if t > 0 else 0.0, zl[t])
                rt = jnp.where(lane == 127, zr[t + 1] if t < NT - 1 else 0.0, zr[t])
                out.append(z[1][t] + lt + rt)
            return out, z[1]

        def fold4(v):
            s = lax.broadcasted_iota(jnp.int32, (8, 128), 0)
            m4 = s < 4
            m2 = (s & 2) == 0
            a = jnp.where(m4, v[0], v[1]) + pltpu.roll(jnp.where(m4, v[1], v[0]), 4, 0)
            b = jnp.where(m4, v[2], v[3]) + pltpu.roll(jnp.where(m4, v[3], v[2]), 4, 0)
            w = jnp.where(m2, a + pltpu.roll(a, 6, 0), b + pltpu.roll(b, 2, 0))
            return w + pltpu.roll(w, 7, 0)

        def stats(acc, y):
            if acc is None:
                return y, [b * b for b in y]
            return [a + b for a, b in zip(acc[0], y)], [a + b * b for a, b in zip(acc[1], y)]

        def put_rstd(ref, r, acc):
            m = fold4(acc[0]) * (1.0 / C)
            q = fold4(acc[1]) * (1.0 / C)
            rs = lax.rsqrt(jnp.maximum(q - m * m, 0.0) + _EPS)
            ref[U, (r % 12) * 8:(r % 12) * 8 + 8, 128 + 128 * (r // 12):256 + 128 * (r // 12)] = rs

        def gelu(z):
            t = z * (z * z + _C0)
            return z * jnp.tanh(t) + z

        def rev(g, kk):
            return jnp.concatenate([g[kk * 128 + j * 8:kk * 128 + j * 8 + 8] for j in reversed(range(16))], axis=0)

        def parked(v, kk):
            if kk < NK - 1:
                return v
            return jnp.concatenate([gelu(v[:_RAW_CHUNKS * 8]), v[_RAW_CHUNKS * 8:]], axis=0)

        for j in range(3):
            zs[j] = 0
        head0 = pltpu.make_async_copy(x_hbm.at[pl.ds(0, _HEAD)], xbuf.at[3, pl.ds(0, _HEAD)], xsem.at[3])
        head1 = pltpu.make_async_copy(x_hbm.at[pl.ds(_HEAD, U - _HEAD)], xbuf.at[3, pl.ds(_HEAD, U - _HEAD)], xsem.at[2])
        head2 = pltpu.make_async_copy(x_hbm.at[pl.ds(U, LA - U)], obuf.at[3, pl.ds(0, LA - U)], osem.at[3])
        cdw, cw1, cb1, cw2, cb2, cg_ = [
            pltpu.make_async_copy(a, b, psem.at[n]) for n, (a, b) in enumerate(
                [(dw_hbm, dw_ref), (w1_hbm, w1_ref), (b1_hbm, b1_ref), (w2t_hbm, w2t_ref), (b2_hbm, b2_ref), (g_hbm, g_ref)])]
        for c in (cdw, cw1, cb1, cw2, cb2, cg_, head0):
            c.start()
        gs[...] = jnp.zeros(gs.shape, F32)
        xr[0] = jnp.zeros((C, W), F32)
        xr[1] = jnp.zeros((C, W), F32)
        for c in (cdw, cb2, cg_):
            c.wait()
        head1.start()
        head2.start()
        dw2_ref[...] = dw_ref[...]

        rows = [(dw2_ref if a == 0 else dw_ref)[a, b:b + 1, :].astype(F32) for a in range(3) for b in range(3)]
        rows += [b2_ref[...].astype(F32), g_ref[...].astype(F32)]
        p = jnp.concatenate(rows + [jnp.zeros((128 - len(rows), C), F32)], axis=0)
        pt = jnp.concatenate([p, jnp.zeros((128, 128 - C), F32)], axis=1).T
        for k in range(9):
            xf[k // 4, :, (k % 4) * 128:(k % 4) * 128 + 128] = jnp.broadcast_to(pt[:C, k:k + 1], (C, 128))
        gcol = pt[:C, 10:11]
        xf[3, :, 0:128] = jnp.broadcast_to(pt[:C, 9:10] * gcol, (C, 128))

        head0.wait()
        for c in (cw1, cb1, cw2):
            c.wait()
        w2f = (w2t_ref[...].astype(F32) * (gcol * (0.5 / _A))).astype(BF16)
        for k in range(NK):
            w2s[k] = pltpu.bitcast(w2f[:, k * 128:(k + 1) * 128], U32)
        w1 = w1_ref[...].astype(F32)
        w1c = (w1 - jnp.mean(w1, axis=0, keepdims=True)) * _A
        b1 = b1_ref[...].astype(F32).reshape(1, E) * _A
        b1h = b1.astype(BF16).astype(F32)
        r8 = lax.broadcasted_iota(jnp.int32, (8, E), 0)
        tail = jnp.where(r8 == 0, b1h, jnp.where(r8 == 1, b1 - b1h, 0.0))
        wt = jnp.concatenate([w1c, tail, jnp.zeros((128 - C - 8, E), F32)], axis=0).T
        wt = jnp.concatenate([rev(wt, kk) for kk in range(NK)], axis=0)
        w1s[0] = pltpu.bitcast(wt.astype(BF16), U32)

        acc = {}
        for q0 in range(0, U, _PRO):
            if q0 <= _HEAD < q0 + _PRO + 1:
                head1.wait()
                head2.wait()
                xchunk(0).start()
                xchunk(1).start()
            for cgi in range(NCG):
                cs = slice(cgi * 8, cgi * 8 + 8)

                def row(r):
                    if r < 0:
                        return jnp.zeros((8, W), F32)
                    v = (xbuf[3, r, cs, :] if r < U else obuf[3, r - U, cs, :]).astype(F32)
                    xr[r + 2, cs, :] = v
                    return v
                xs = {r: row(r) for r in range(q0 - 1, q0 + _PRO + 1)}
                if q0 + _PRO == U:
                    for r in range(U + 1, LA):
                        row(r)
                for r in range(q0, q0 + _PRO):
                    y, _ = conv(cgi, [xs[r - 1], xs[r], xs[r + 1]], xf)
                    ya[r, cs, :] = jnp.concatenate(y, axis=1)
                    acc[r] = stats(acc.get(r), y)
            for r in range(q0, q0 + _PRO):
                put_rstd(ya, r, acc[r])

        def block(k, par, ycur, ynxt):
            r0 = k * U
            z0, z1, z2 = zs[0], zs[1], zs[2]
            src = xbuf.at[k % 4]
            ocur = obuf.at[k % 4]
            onxt = obuf.at[(k + 1) % 4]
            wd = xf.at[pl.ds(z0, 4)]
            ybd = ycur.at[pl.ds(z0, U + 1)]

            def ring(r):
                return (par * U + r + 2) % RING

            ev = []
            st = dict(n=0, acc=None, up=LA, z=None)
            vals = {}

            def token(T, wide=False):
                c = [e for e in ev if e[0] <= T + 1e-6]
                if not c:
                    return None
                _, a, j = max(c, key=lambda e: e[0])
                return a[j * 8:j * 8 + 8, 0:256].astype(BF16) if wide else a[j * 8:j * 8 + 8, 0:128]

            def run(T, kind, u, h, n):
                if kind == "conv":
                    v, n = divmod(st["n"], NCG)
                    if v >= U:
                        return
                    assert v + U + 1 < st["up"]
                    t_ = token(T)
                    if t_ is None:
                        t_ = st["z"]
                    if t_ is not None:
                        xf[3 + z2, 0:8, 384:512] = t_
                    cs = slice(n * 8, n * 8 + 8)
                    y, zc = conv(n, [xr[ring(v + U - 1 + q), cs, :] for q in range(3)], wd)
                    st["z"] = zc[2]
                    ynxt[v, cs, :] = jnp.concatenate(y, axis=1)
                    st["acc"] = stats(st["acc"] if n else None, y)
                    if n == NCG - 1:
                        put_rstd(ynxt, v, st["acc"])
                    st["n"] += 1
                elif kind == "unpack":
                    v = token(T, True) if T <= 8 else None
                    if v is not None:
                        xbuf[4 + z1, 0, 0:8, 0:256] = v
                    cs = slice(n * (C // NUP), (n + 1) * (C // NUP))
                    xr[ring(st["up"]), cs, :] = src[u, cs, :].astype(F32)
                    if n == NUP - 1:
                        st["up"] += 1
                elif kind == "rhs":
                    v = token(T)
                    if v is not None:
                        ycur[U + z1, 0:8, 0:128] = v
                    if ("rs", u) not in vals:
                        vals["rs", u] = ybd[U, (u % 12) * 8:(u % 12) * 8 + 8, 128 + 128 * (u // 12):256 + 128 * (u // 12)]
                    t = 2 * h + n
                    sl = (0, 4, 2, 6)[t]
                    vals["h", u, t] = ybd[u, :, t * 128:(t + 1) * 128] * vals["rs", u][sl:sl + 1, :]
                elif kind == "w1":
                    v = token(T)
                    if v is not None:
                        w1s[1 + z1, 0:8, :] = pltpu.bitcast(v, U32)
                    vals["w1", u, h] = w1s[0, 0:E // 2, :]
                elif kind == "w2":
                    v = token(T)
                    if v is not None:
                        w2s[NK + z1, 0:8, :] = pltpu.bitcast(v, U32)
                    vals["w2", u, h, n] = w2s[n + z0]
                elif kind == "load":
                    v = token(T)
                    if v is not None:
                        gs[E + z1 * 8:E + z1 * 8 + 8, 0:128] = v
                    vals["g", u, h, n] = parked(gs[pl.ds(pl.multiple_of(z0 * 8 + n * 128, 8), 128), :], n)
                elif kind == "park":
                    m = (n // 16) * 16 + 15 - n % 16
                    gs[m * 8:m * 8 + 8, :] = vals["graw" if n < 48 - _RAW_CHUNKS else "zraw"][n * 8:n * 8 + 8, :]
                elif kind == "out":
                    token(T)
                    nr = C // _OUT_PIECES
                    rs8 = slice(n * nr, n * nr + nr)
                    hs = slice(h * HW, h * HW + HW)
                    gbv = tap(wd, 12, rs8)
                    res = xr[ring(u), rs8, hs] + jnp.concatenate([gbv, gbv], axis=1)
                    P = vals["P", u, h]
                    out = (((P[0][rs8] + P[1][rs8]) + res) + P[2][rs8]).astype(o_hbm.dtype)
                    if u + 1 < U:
                        ocur[u + 1, rs8, hs] = out
                    else:
                        onxt[0, rs8, hs] = out

            items, lhs1 = [], {}

            def add(T, kind, u, h, n):
                items.append((T, len(items), kind, u, h, n))

            def m1start(u, h):
                return 42 * u + 18.0 * h

            def m2start(u, h):
                return 42 * u + (24 if h == 0 else 42)

            for u in range(-1, U):
                if u >= 0:
                    for tau in _CONV["first" if u == 0 else "last" if u == U - 1 else "mid"]:
                        add(42 * u + tau, "conv", u, 0, 0)
                    for n in range(NUP):
                        add(42 * u + _UNPACK[n], "unpack", u, 0, n)
                for h in range(2):
                    if u >= 0:
                        for n in range(2):
                            add(m1start(u, h) - _RHS_LEAD[h][n], "rhs", u, h, n)
                        lhs1[u, h] = (m1start(u, h) - _W1_LEAD[h], "w1", u, h, 0)
                    if u == U - 1 and h == 1:
                        for j in range(48):
                            add(42 * u + 27 + j / 2, "park", u, h, j)
                        continue
                    if u == -1 and h == 0:
                        continue
                    m2 = m2start(u, h)
                    for kk in range(NK):
                        add(m2 + 6 * kk - _W2_LEAD[3 * h + kk], "w2", u, h, kk)
                        if u == -1:
                            add(m2 + 6 * kk - _PARK_LEAD, "load", u, h, kk)
                    for q in range(_OUT_PIECES):
                        add(m2 + 20 + q * 6.0 / _OUT_PIECES + _OUT_OFF + _OUT_SKEW * q, "out", u, h, q)
            items.sort()
            done = [0]

            def flush(pred):
                last = max([i for i, it in enumerate(items) if pred(it)], default=-1)
                while done[0] <= last:
                    T, _, kind, u, h, n = items[done[0]]
                    run(T, kind, u, h, n)
                    done[0] += 1

            def mat1(u, h):
                flush(lambda it: it[2] == "rhs" and it[3] == u and it[4] == h)
                run(*lhs1[u, h])
                lhs = jnp.concatenate([vals["w1", u, h]], axis=0)
                hn = jnp.concatenate([vals["h", u, 2 * h], vals["h", u, 2 * h + 1]], axis=1)
                s8 = lax.broadcasted_iota(jnp.int32, (8, HW), 0)
                ones = jnp.where(s8 < 2, 1.0, 0.0).astype(F32)
                z = mm(pltpu.bitcast(lhs, BF16),
                       jnp.concatenate([hn, ones, jnp.zeros((128 - C - 8, HW), F32)], axis=0))
                g = gelu(z)
                vals["graw"], vals["zraw"] = g, z
                for kk in range(NK):
                    vals["g", u, h, kk] = rev(g, kk)
                ev.extend((m1start(u, h) + 9 + j / 2, g, j) for j in range(48))

            def mat2(u, h):
                flush(lambda it: it[2] in ("w2", "load") and it[3] == u and it[4] == h)
                P = [mm(pltpu.bitcast(vals["w2", u, h, kk], BF16), vals["g", u, h, kk]) for kk in range(NK)]
                vals["P", u, h] = P
                ev.extend((m2start(u, h) + 8 + 6 * kk + j / 2 + 0.01, P[kk], j) for kk in range(NK) for j in range(12))

            run(-20, "conv", 0, 0, 0)
            for u in range(U):
                mat1(u, 0)
                mat2(u - 1, 1)
                mat1(u, 1)
                if u == U - 1:
                    flush(lambda it: it[2] == "out" and it[3] == u - 1 and it[4] == 1)
                    pl.when(k == 0)(lambda: ofirst.start())
                    pl.when(k > 0)(lambda: ochunk(k).start())
                mat2(u, 0)
            flush(lambda it: True)
            assert st["n"] == U * NCG and st["up"] == LA + U

        def body(k, carry):
            @pl.when(k + 2 < KP)
            def _():
                xchunk(k).wait()
                xchunk(k + 2).start()

            @pl.when(k + 2 >= KP)
            def _():
                pl.when(k < KP)(lambda: xchunk(k).wait())

                @pl.when(k == KP)
                def _():
                    xpart().wait()
                    xbuf[KP % 4, NP] = jnp.zeros((C, W), BF16)

                pl.when(k + 2 == KP)(lambda: xpart().start())

            pl.when((k & 1) == 0)(lambda: block(k, 0, ya, yb))
            pl.when((k & 1) == 1)(lambda: block(k, 1, yb, ya))
            pl.when(k > 2)(lambda: ochunk(k - 2).wait())
            pl.when(k == 2)(lambda: ofirst.wait())
            return carry

        lax.fori_loop(0, NBLK, body, 0)

        out = xr[(H - 1 + 2) % RING, :, HW:] + jnp.concatenate([tap(xf, 12, slice(0, C))] * 2, axis=1)
        for kk in range(NK):
            out = out + mm(pltpu.bitcast(w2s[kk], BF16), parked(gs[kk * 128:(kk + 1) * 128, :], kk))
        obuf[NBLK % 4, 0, :, HW:] = out.astype(o_hbm.dtype)
        olast.start()
        ochunk(NBLK - 2).wait()
        ochunk(NBLK - 1).wait()
        olast.wait()

    scratch = [
        pltpu.VMEM((9, U, C, W), BF16),
        pltpu.SemaphoreType.DMA((4,)),
        pltpu.SemaphoreType.DMA((4,)),
        pltpu.VMEM((2, E // 2, 128), U32),
        pltpu.VMEM((NK + 1, C // 2, 128), U32),
        pltpu.VMEM((4, C, W), F32),
        pltpu.VMEM((RING, C, W), F32),
        pltpu.VMEM((U + 1, C, W), F32),
        pltpu.VMEM((U + 1, C, W), F32),
        pltpu.VMEM((E + 8, HW), F32),
        pltpu.SMEM((3,), jnp.int32),
    ]
    return kernel, scratch


@jax.jit
def pallas_standalone__modern_conv_block_convnext__vision_kernel(x, dw, w1, b1, w2, b2, gamma):
    B, H, W, C = x.shape
    E = w1.shape[1]
    assert B == 1 and dw.shape[:2] == (3, 3)
    xt = jnp.transpose(x[0], (0, 2, 1))
    args = (dw, w1, b1, w2.T, b2.reshape(1, C), gamma.reshape(1, C))
    kernel, scratch = _make_kernel(H, C, W, E)
    scratch += [pltpu.VMEM(args[n].shape, args[n].dtype) for n in (1, 3, 0, 2, 4, 5)]
    scratch += [pltpu.SemaphoreType.DMA((len(args),)), pltpu.VMEM(dw.shape, dw.dtype)]
    hbm = pl.BlockSpec(memory_space=pl.ANY)
    out = pl.pallas_call(
        kernel,
        in_specs=[hbm] * (1 + len(args)),
        out_specs=hbm,
        out_shape=jax.ShapeDtypeStruct((H, C, W), x.dtype),
        scratch_shapes=scratch,
        compiler_params=pltpu.CompilerParams(
            vmem_limit_bytes=96 * 1024 * 1024,
            disable_bounds_checks=True,
            flags={"XLA_TPU_EVENLY_DISTRIBUTE_CRITICAL_NODES": True},
        ),
    )(xt, *args)
    return jnp.transpose(out, (0, 2, 1))[None]
```
